```python
import os as _os
_os.environ.setdefault("JAX_PLATFORMS", "cpu")
import jax
import jax.numpy as jnp

def _softmax(x, axis=-1):
    return jax.nn.softmax(x, axis=axis)
def _gelu(x):
    return jax.nn.gelu(x, approximate=True)
def _silu(x):
    return jax.nn.silu(x)
def _sigmoid(x):
    return jax.nn.sigmoid(x)
def _layernorm(x, axis=-1, eps=1e-5):
    m = jnp.mean(x, axis=axis, keepdims=True)
    v = jnp.var(x, axis=axis, keepdims=True)
    return (x - m) / jnp.sqrt(v + eps)
def _scatter_add(tgt, idx, src, axis=0):
    return tgt.at[idx].add(src)
def _segment_sum(src, seg, n):
    return jax.ops.segment_sum(src, seg, n)
class _Rng:
    def __init__(self, key):
        self._k = key
    def _next(self):
        self._k, sub = jax.random.split(self._k)
        return sub
    def normal(self, shape):
        return jax.random.normal(self._next(), shape, dtype=jnp.bfloat16)
    def randint(self, lo, hi, shape):
        return jax.random.randint(self._next(), shape, lo, hi, dtype=jnp.int32)
    def uniform(self, shape, lo=0.0, hi=1.0):
        return jax.random.uniform(self._next(), shape, jnp.bfloat16, lo, hi)
    def permutation(self, n):
        return jax.random.permutation(self._next(), n)


kernel_name = 'parallel_sum__softmax_full_mha__glu_gated_swiglu__prompt'

def setup_inputs():
    _rng = _Rng(jax.random.key(int.from_bytes(__import__("os").urandom(4), "little")))
    _w = (lambda a: (lambda t: t.astype(jnp.bfloat16) if jnp.issubdtype(t.dtype, jnp.floating) else t)(jnp.asarray(a)))
    def _A_setup():
        B, S, D = 1, 2048, 448
        return {
            "x": _w((lambda *s: _rng.normal(s) * 0.05)(B, S, D)),
            "wqkv": _w((lambda *s: _rng.normal(s) * 0.05)(D, 3 * D)),
            "wo": _w((lambda *s: _rng.normal(s) * 0.05)(D, D)),
        }
    _A_in = _A_setup()

    def _B_setup():
        B, S, D, F = 1, 2048, 448, 1792
        return {
            "x": _w((lambda *s: _rng.normal(s) * 0.05)(B, S, D)),
            "w1": _w((lambda *s: _rng.normal(s) * 0.05)(D, F) * (2.0 / D) ** 0.5),
            "w3": _w((lambda *s: _rng.normal(s) * 0.05)(D, F) * (2.0 / D) ** 0.5),
            "w2": _w((lambda *s: _rng.normal(s) * 0.05)(F, D) * (2.0 / F) ** 0.5),
        }
    _B_in = _B_setup()

    return {
        "A_x": _A_in["x"],
        "A_wqkv": _A_in["wqkv"],
        "A_wo": _A_in["wo"],
        "B_x": _B_in["x"],
        "B_w1": _B_in["w1"],
        "B_w3": _B_in["w3"],
        "B_w2": _B_in["w2"],
    }

def reference(A_x, A_wqkv, A_wo, B_x, B_w1, B_w3, B_w2):
    def _A_ref(x, wqkv, wo):
        B, S, D = x.shape
        H = 16; Dh = D // H
        qkv = (lambda x, *d: x.transpose(*d))((x @ wqkv).reshape(B, S, 3, H, Dh), 2, 0, 3, 1, 4)
        q, k, v = qkv[0], qkv[1], qkv[2]
        scale = Dh ** -0.5
        scores = jnp.einsum("bhqd,bhkd->bhqk", q, k) * scale
        p = _softmax(scores, axis=-1)
        o = jnp.einsum("bhqk,bhkd->bhqd", p, v)
        return (lambda x, *d: x.transpose(*d))(o, 0, 2, 1, 3).reshape(B, S, D) @ wo

    def _B_ref(x, w1, w3, w2):
        gate = jnp.einsum("bsd,df->bsf", x, w1)
        up = jnp.einsum("bsd,df->bsf", x, w3)
        h = _silu(gate) * up
        out = jnp.einsum("bsf,fd->bsd", h, w2)
        return out

    x = A_x
    xn = _layernorm(x, axis=-1)
    return x + _A_ref(xn, A_wqkv, A_wo) + _B_ref(xn, B_w1, B_w3, B_w2)
```

```python
import functools
import math

import jax
import jax.numpy as jnp
from jax import lax
from jax.experimental import pallas as pl
from jax.experimental.pallas import tpu as pltpu

S, D, H, F = 2048, 448, 16, 1792
DH = D // H
HP = 32
TQ = 512
NT = S // TQ
CH = 128
EPS = 1e-5
QSCALE = DH ** -0.5 * math.log2(math.e)

f32, bf16 = jnp.float32, jnp.bfloat16


def _dot(a, b):
    return jnp.dot(a, b, preferred_element_type=f32)


def _head_window(h):
    lo = DH * h
    return (lo, 0) if h % 2 == 0 else (lo - (HP - DH), HP - DH)


def make_kernel(unroll_heads=True):
    def kernel(xT_hbm, wqkv_hbm, wo_hbm, w1_hbm, w3_hbm, w2T_hbm, outT_hbm,
               xT, wqkv, wo, w1, w3, w2T,
               wqkvT, w1T, w3T, woT,
               xnT, qT, kk, vT, hT, oT, s0, s1, outb,
               x_sem, w_sem, o_sem):
        def x_copy(c):
            return pltpu.make_async_copy(
                xT_hbm.at[:, pl.ds(c * TQ, TQ)], xT.at[c], x_sem.at[c])

        w_copies = [
            pltpu.make_async_copy(src, dst, w_sem.at[i])
            for i, (src, dst) in enumerate(
                [(wqkv_hbm, wqkv), (w1_hbm, w1), (w3_hbm, w3), (wo_hbm, wo), (w2T_hbm, w2T)])
        ]
        x_copy(0).start()
        w_copies[0].start()
        for c in range(1, NT):
            x_copy(c).start()
        for cp in w_copies[1:]:
            cp.start()

        row32 = lax.broadcasted_iota(jnp.int32, (HP, TQ), 0)

        def project(c):
            x = xT[c].astype(f32)
            mean = jnp.sum(x, axis=0, keepdims=True) * (1.0 / D)
            xc = x - mean
            var = jnp.sum(xc * xc, axis=0, keepdims=True) * (1.0 / D)
            xn = (xc * lax.rsqrt(var + EPS)).astype(bf16)
            xnT[c] = xn
            k = _dot(wqkvT[pl.ds(D, D), :], xn).astype(bf16)
            kpad = jnp.concatenate([k, jnp.zeros((16, TQ), bf16)], axis=0)
            for j in range(4):
                kk[j, pl.ds(c * TQ, TQ), :] = kpad[112 * j:112 * j + 128].T
            q = _dot(wqkvT[pl.ds(0, D), :], xn) * QSCALE
            qT[c] = q.astype(bf16)
            v = _dot(wqkvT[pl.ds(2 * D, D), :], xn)
            for h in range(H):
                lo, d0 = _head_window(h)
                win = v[lo:lo + HP]
                if d0 == 0:
                    win = jnp.where(row32 < DH, win, jnp.where(row32 == DH, 1.0, 0.0))
                else:
                    win = jnp.where(row32 >= d0, win, jnp.where(row32 == 0, 1.0, 0.0))
                vT[h, :, pl.ds(c * TQ, TQ)] = win.astype(bf16)

        x_copy(0).wait()
        w_copies[0].wait()
        wqkvT[...] = wqkv[...].T
        project(0)
        x_copy(1).wait()
        project(1)
        x_copy(2).wait()
        w_copies[1].wait()
        w1T[...] = w1[...].T
        project(2)
        x_copy(3).wait()
        w_copies[2].wait()
        w_copies[3].wait()
        w3T[...] = w3[...].T
        wof = wo[...].astype(f32)
        rowo = lax.broadcasted_iota(jnp.int32, (HP, D), 0)
        pieces = []
        for h in range(H):
            lo, d0 = _head_window(h)
            win = wof[lo:lo + HP]
            pieces.append(jnp.where((rowo >= d0) & (rowo < d0 + DH), win, 0.0))
        woT[...] = jnp.concatenate(pieces, axis=0).astype(bf16).T
        project(3)
        w_copies[4].wait()

        def out_copy(t):
            return pltpu.make_async_copy(
                outb.at[t], outT_hbm.at[:, pl.ds(pl.multiple_of(t * TQ, TQ), TQ)], o_sem.at[t])

        def tile(t, carry):
            sbuf = (s0, s1)
            wsl = t % 2
            rsl = 1 - (t + 1) % 2

            def q_weights(h):
                j, i = divmod(h, 4)
                lo, hi = DH * i, DH * (i + 1)
                a, b = lo // 16 * 16, -(-hi // 16) * 16
                blk = qT[t, pl.ds(112 * j + a, b - a), :]
                r = lax.broadcasted_iota(jnp.int32, (b - a, TQ), 0) + a
                blk = jnp.where((r >= lo) & (r < hi), blk.astype(f32), 0.0).astype(bf16)
                parts = []
                if a:
                    parts.append(jnp.zeros((a, TQ), bf16))
                parts.append(blk)
                parts.append(jnp.zeros((128 - b, TQ), bf16))
                return jnp.concatenate(parts, axis=0)

            def scores(h, qw, c0):
                s = _dot(kk[h // 4, pl.ds(c0, CH), :], qw)
                sbuf[h % 2][wsl, pl.ds(c0, CH), :] = s
                return jnp.max(s.reshape(CH // 8, 8, TQ), axis=0)

            def values(h, m, c0):
                p = jnp.exp2(sbuf[h % 2][rsl, pl.ds(c0, CH), :] - m).astype(bf16)
                return _dot(vT[h, :, pl.ds(c0, CH)], p)

            def finish(h, acc):
                _, d0 = _head_window(h)
                lrow = DH if d0 == 0 else 0
                oT[pl.ds(HP * h, HP), :] = (acc / acc[lrow:lrow + 1]).astype(bf16)

            def gate_up(r0, n):
                g = _dot(w1T[pl.ds(r0, n), :], xnT[t])
                u = _dot(w3T[pl.ds(r0, n), :], xnT[t])
                hT[pl.ds(r0, n), :] = (g * u / (1.0 + jnp.exp(-g))).astype(bf16)

            m = None
            y = xT[t].astype(f32)
            for h in range(H + 1):
                if h < H:
                    qw = q_weights(h)
                mx, acc = None, None
                for ci, c0 in enumerate(range(0, S, CH)):
                    if h < H:
                        mm = scores(h, qw, c0)
                        mx = mm if mx is None else jnp.maximum(mx, mm)
                    elif ci < F // 128:
                        y = y + _dot(w2T[:, pl.ds(128 * ci, 128)], hT[pl.ds(128 * ci, 128), :])
                    if h > 0:
                        o = values(h - 1, m, c0)
                        acc = o if acc is None else acc + o
                if h < F // 128:
                    gate_up(128 * h, 128)
                if h > 0:
                    finish(h - 1, acc)
                if h < H:
                    m = jnp.max(mx, axis=0, keepdims=True)
            y = y + _dot(woT[...], oT[...])
            outb[t] = y.astype(bf16)
            out_copy(t).start()
            return carry

        lax.fori_loop(0, NT, tile, 0)
        for t in range(NT):
            out_copy(t).wait()

    return kernel


def build(**kw):
    flags = kw.pop("flags", None)
    name = kw.pop("name", "fused_block")

    def run(A_x, A_wqkv, A_wo, B_x, B_w1, B_w3, B_w2):
        del B_x
        hbm = pl.BlockSpec(memory_space=pltpu.HBM)
        vm = pltpu.VMEM
        outT = pl.pallas_call(
            make_kernel(**kw),
            out_shape=jax.ShapeDtypeStruct((D, S), bf16),
            in_specs=[hbm] * 6,
            out_specs=hbm,
            scratch_shapes=[
                vm((NT, D, TQ), bf16), vm((D, 3 * D), bf16), vm((D, D), bf16),
                vm((D, F), bf16), vm((D, F), bf16), vm((D, F), bf16),
                vm((3 * D, D), bf16), vm((F, D), bf16), vm((F, D), bf16), vm((D, H * HP), bf16),
                vm((NT, D, TQ), bf16), vm((NT, D, TQ), bf16), vm((4, S, 128), bf16),
                vm((H, HP, S), bf16), vm((F, TQ), bf16), vm((H * HP, TQ), bf16),
                vm((2, S, TQ), f32), vm((2, S, TQ), f32), vm((NT, D, TQ), bf16),
                pltpu.SemaphoreType.DMA((NT,)), pltpu.SemaphoreType.DMA((5,)),
                pltpu.SemaphoreType.DMA((NT,)),
            ],
            compiler_params=pltpu.CompilerParams(vmem_limit_bytes=100 * 2**20, flags=flags),
            name=name,
        )(A_x[0].T, A_wqkv, A_wo, B_w1, B_w3, B_w2.T)
        return outT.T[None]

    return jax.jit(run, keep_unused=True)


_run = build()


@jax.jit
def pallas_parallel_sum__softmax_full_mha__glu_gated_swiglu__prompt_kernel(
    A_x, A_wqkv, A_wo, B_x, B_w1, B_w3, B_w2
):
    return _run(A_x, A_wqkv, A_wo, B_x, B_w1, B_w3, B_w2)
```

```python
import contextlib
import math

import jax
import jax.numpy as jnp
from jax import lax
from jax.experimental import pallas as pl
from jax.experimental.pallas import tpu as pltpu

S, D, H, F = 2048, 448, 16, 1792
DH = D // H
HP = 32
TQ = 256
TH = TQ // 2
NT = S // TQ
NP = H // 2
D2, D4, F2 = D // 2, D // 4, F // 2
KH = 192
RG = 64
NU = 25
EPS = 1e-5
QSCALE = DH ** -0.5 * math.log2(math.e)

f32, bf16, u32 = jnp.float32, jnp.bfloat16, jnp.uint32


def _dot(a, b):
    return jnp.dot(a, b, preferred_element_type=f32)


def _pack(x):
    return pltpu.bitcast(x.astype(bf16), u32)


def _unpack(x):
    return pltpu.bitcast(x, bf16)


def _rows(start, n):
    return pl.ds(start // 2, n // 2)


def _head_window(e):
    return (0, 0) if e == 0 else (2 * DH - HP, HP - DH)


def _split(x):
    return [pltpu.unpack_elementwise(x, index=i, packed_dtype=bf16, unpacked_dtype=f32) for i in range(2)]


def _join(x):
    return pltpu.pack_elementwise(x, packed_dtype=bf16)


def _add(x, y):
    return [a + b for a, b in zip(x, y)]


def _sub(x, y):
    return [a - b for a, b in zip(x, y)]


def _lhs_operands(a11, a12, a21, a22):
    x11, x12, x21, x22 = (_split(a) for a in (a11, a12, a21, a22))
    return [_join(_add(x11, x22)), _join(_add(x21, x22)), a11, a22,
            _join(_add(x11, x12)), _join(_sub(x21, x11)), _join(_sub(x12, x22))]


def _rhs_operands(b11, b12, b21, b22):
    return [b11 + b22, b11, b12 - b22, b21 - b11, b22, b11 + b12, b21 + b22]


ORDER = (2, 3, 4, 1, 0, 6, 5)
SHARED = {0: (0, 3), 1: (2, 3), 4: (0, 1)}
REMAINDER = {2: 1, 3: 0, 5: 1, 6: 0}
PASSES = [(i, k) for i in ORDER
          for k in ([(0, 1), (2, 1), (0, 2)] if i in SHARED else [(0, 1), (2, 3), (0, 1), (3, 2)])]


def _combine(m):
    m1, m2, m3, m4, m5, m6, m7 = (m[i] for i in range(7))
    return m7 + (m1 + (m4 - m5)), m3 + m5, m4 + m2, m6 + (m1 + (m3 - m2))


def _pass_weights(p, q):
    low = lax.broadcasted_iota(jnp.int32, p[0][0].shape, 1) < 64
    ops = [[_lhs_operands(*x[k]) for k in range(2)] for x in (p, q)]
    out = []
    for i in ORDER:
        (p0, p1), (q0, q1) = ([x[k][i] for k in range(2)] for x in ops)
        if i in SHARED:
            diff = _join(_sub(*(_add(*(_split(x[0][b]) for b in SHARED[i])) for x in (p, q))))
            out += [jnp.where(low, p0, q0), jnp.where(low, p1, diff), jnp.where(low, diff ^ jnp.uint32(0x80008000), q1)]
        else:
            out += [p0, p1, q0, q1]
    return out


def _collect(r):
    r, mp, mq = list(r), {}, {}
    for i in ORDER:
        if i in SHARED:
            both, own_p, own_q = r.pop(0), r.pop(0), r.pop(0)
            mp[i], mq[i] = own_p + both, own_q + both
        else:
            p0, p1, q0, q1 = r.pop(0), r.pop(0), r.pop(0), r.pop(0)
            mp[i], mq[i] = p1 + p0, q1 + q0
    cp, cq = _combine(mp), _combine(mq)
    return [cp[:2], cq[:2], cp[2:], cq[2:]]


def _assemble(blocks):
    return jnp.concatenate([jnp.concatenate(list(b), 1) for b in blocks], 0)


def make_kernel(VT=6, KB=2, wq0=64, wq=38, wv=38, wg=54, wd=54, every=1, ntie=2, slack=20, KG=7,
                waits=(4, 11, 17), starts=(2, 8), xl=12, tied2='ze in ut', pu=0, opq='', tl=2.5, tailg=8, spread=True, insv=2, ymem=True, pstep=1, rel=0, qunit=3, short=True, tu=0, four=False, gsteps=12, mid=(), hlag=10, wact=11, hmem=2, htie=(5, 6), TU=2,
                scopes=False, noprol=False, nomain=False):
    VR = 16

    def scope(name):
        return jax.named_scope(name) if scopes else contextlib.nullcontext()

    def kernel(xT_hbm, wqkv_hbm, wo_hbm, w1_hbm, w3_hbm, w2T_hbm, outT_hbm,
               xT, wqkv, wo, w1, w3, w2T,
               wT, fT, aqkv, a13, a2,
               xB, qf, kk, kb0, kb1, vT, oF, s0, s1, sv, m0, m1, yb, hB, yacc, outb,
               x_sem, w_sem, o_sem):
        def x_copy(t):
            return pltpu.make_async_copy(
                xT_hbm.at[:, pl.ds(t * TQ, TQ)], xT.at[t], x_sem.at[t])

        def w_copy(i):
            src, dst = [(wqkv_hbm, wqkv), (w2T_hbm, w2T), (w1_hbm, w1), (wo_hbm, wo), (w3_hbm, w3)][i]
            return pltpu.make_async_copy(src, dst, w_sem.at[i])

        def tiles(*xs):
            return [x[r:r + 8, c:c + 128] for x in xs
                    for r in range(0, x.shape[0], 8) for c in range(0, x.shape[1], 128)]

        def tie(x, deadline, never):
            rows = []
            for r in range(0, x.shape[0], 8):
                first = x[r:r + 8, :128]
                for k, dep in enumerate(deadline()):
                    first = jnp.where(never[k], pltpu.bitcast(dep, u32), first)
                rows.append(first if x.shape[1] == 128 else jnp.concatenate([first, x[r:r + 8, 128:]], 1))
            return _unpack(jnp.concatenate(rows, 0))

        def operand(src, n):
            i, pieces = PASSES[n]
            return _unpack(jnp.concatenate(
                [src[i, _rows(64 * k, 64), :] if k < 3 else src[7, _rows(64 * REMAINDER[i], 64), :]
                 for k in pieces], 0))

        def stage(dst, n, res):
            i = PASSES[n][0]
            if i in SHARED and len(res) > 1:
                dst[len(res) - 2, i] = res[-1] + res[0]
            elif i not in SHARED and len(res) % 2 == 0:
                dst[len(res) // 2 - 1, i] = res[-1] + res[-2]
            return [] if len(res) == (3 if i in SHARED else 4) else res

        def normalize(t):
            acc = 0.0
            for r in range(0, D, 64):
                acc = acc + jnp.sum(xT[t, pl.ds(r, 64), :].astype(f32).reshape(8, 8, TQ), axis=0)
                yield tiles(acc)
            mean = jnp.sum(acc, axis=0, keepdims=True) * (1.0 / D)
            acc = 0.0
            for r in range(0, D, 32):
                xc = xT[t, pl.ds(r, 32), :].astype(f32) - mean
                acc = acc + jnp.sum((xc * xc).reshape(4, 8, TQ), axis=0)
                yield tiles(acc)
            scale = lax.rsqrt(jnp.sum(acc, axis=0, keepdims=True) * (1.0 / D) + EPS)
            yield []

            def block(r):
                return [(x - mean) * scale for x in _split(_pack(xT[t, pl.ds(r, 16), :]))]

            for r in range(0, KH, 16):
                ops = [_rhs_operands(a[:, :TH], a[:, TH:], b[:, :TH], b[:, TH:]) + [a[:, TH:], b[:, :TH]]
                       for a, b in zip(block(r), block(KH + r))]
                ops = [_join(list(x)) for x in zip(*ops)]
                for i in range(9):
                    xB[t, i + i // 7, _rows(r, 16), :] = ops[i]
                yield [ops[i] for i in (0, 2, 3, 5, 6)]
            for r in range(0, 64, 16):
                rest = _join(block(2 * KH + r))
                for u in range(2):
                    xB[t, 7, _rows(64 * u + r, 16), :] = rest[:, u * TH:(u + 1) * TH]
                yield tiles(rest)

        row32 = lax.broadcasted_iota(jnp.int32, (HP, TQ), 0)

        def store_q(t, p, blk):
            qf[p, t, pl.ds(0, 2 * DH), :] = blk * QSCALE

        def store_k(t, p, blk):
            gap = jnp.zeros((8, TH), f32)
            both = jnp.concatenate([blk[:, :TH], gap, blk[:, TH:], gap], axis=0)
            kk[p, t] = _pack(both.astype(bf16).T)

        def store_v(t, p, blk):
            for e in range(2):
                lo, d0 = _head_window(e)
                win = blk[lo:lo + HP]
                if d0 == 0:
                    win = jnp.where(row32 < DH, win, jnp.where(row32 == DH, 1.0, 0.0))
                else:
                    win = jnp.where(row32 >= d0, win, jnp.where(row32 == 0, 1.0, 0.0))
                vT[2 * p + e, :, pl.ds(t * TQ, TQ)] = _pack(win)

        def project(pace, t, slot, j, event):
            def rhs(u, *pieces):
                where = ((1, 9), (8, 4))[u]
                return _unpack(jnp.concatenate(
                    [xB[slot, where[k // 3], _rows(64 * (k % 3), 64), :] if k < 6 else xB[slot, 7, _rows(64 * u, 64), :]
                     for k in pieces], 0))

            for m in range(2):
                out = []
                for u in range(2):
                    both = pace.dot(aqkv[j, 7 * m], rhs(u, 0, 1))
                    for inst in range(2):
                        acc = both
                        for n, pieces in enumerate((((2, 1), (0, 2))[inst], (3, 4), (5, 6))):
                            acc = pace.dot(aqkv[j, 7 * m + 1 + 3 * inst + n], rhs(u, *pieces)) + acc
                        out.append(acc)
                full = _assemble([out[0::2], out[1::2]])
                for p in range(NP // 2):
                    (store_q, store_k, store_v)[j](t, NP // 2 * m + p, full[2 * DH * p:2 * DH * (p + 1)])
            event()

        def prep_qkv(j, release):
            skew = j * D % 128
            for c in range(0, D, 128):
                c0 = j * D - skew + c
                n = min(128, 3 * D - c0)
                for x, lo in enumerate((0, 128, 192, 320)):
                    blk = jnp.concatenate([wqkv[pl.ds(r, 64), pl.ds(c0, n)] for r in (lo, lo + (64 if x != 1 else 0))], 0)
                    if release is not None:
                        head = pltpu.bitcast(release(pltpu.bitcast(blk[:16], f32)), bf16)
                        blk = jnp.concatenate([head, blk[16:]], 0)
                    wT[j, x // 2, x % 2, _rows(c, n), :] = _pack(blk.T)
                    yield []
            low = lax.broadcasted_iota(jnp.int32, (D4 // 2, 128), 1) < 64
            for m in range(2):
                p, q = ([wT[j, x // 2, x % 2, _rows(skew + m * D2 + r, D4), :] for x in range(4)] for r in (0, D4))
                diff = _join(_sub(_split(p[0]), _split(q[0])))
                ops = [jnp.where(low, p[0], q[0]), jnp.where(low, p[1], diff), p[2], p[3],
                       jnp.where(low, diff ^ jnp.uint32(0x80008000), q[1]), q[2], q[3]]
                for n, op in enumerate(ops):
                    aqkv[j, 7 * m + n] = op
                yield []

        def spread_keys(p, e, slot, release):
            for t in range(VT):
                for r in range(0, VR, 8):
                    for u in range(2):
                        for d0 in range(0, DH, KG):
                            k = release(_unpack(kk[p, t, _rows(0, VR), :]).astype(f32)[r:r + 8])
                            for d in range(d0, d0 + KG):
                                lane = 64 * u + DH * e + d
                                (kb0, kb1)[e][slot, t, d, pl.ds(u * VR + r, 8), :] = jnp.broadcast_to(
                                    k[:, lane:lane + 1], (8, 128))
                            yield []

        def transposed(w, kind, half, c0, n, release):
            body, rest = half * KH, 2 * KH
            starts = [(body, body + 64), (body + 128, rest), (rest, body + 128)][kind]
            blk = jnp.concatenate([w[pl.ds(r, 64), pl.ds(c0, n)] for r in starts], 0)
            if release is not None:
                head = pltpu.bitcast(release(pltpu.bitcast(blk[:16], f32)), bf16)
                blk = jnp.concatenate([head, blk[16:]], 0)
            return _pack(blk.T)

        def prep_square(j, release):
            w, base = (wqkv, j * D) if j < 3 else (wo, 0)
            skew = base % 128
            for c in range(0, D, 128):
                n = min(128, w.shape[1] - (base - skew + c))
                for kind in range(3):
                    if kind and not any(c < skew + (b + 1) * D4 and skew + b * D4 < c + n for b in (kind - 1, kind + 1)):
                        continue
                    for half in range(2):
                        wT[j, kind, half, _rows(c, n), :] = transposed(w, kind, half, base - skew + c, n, release)
                    yield []
            for _ in range(xl):
                yield []
            for r in range(0, D4, 16):
                p, q = ([[wT[j, kind, half, _rows(skew + inst * D4 + m + r, 16), :] for m in (0, D2) for half in range(2)]
                         for kind in (0, 1 + inst)] for inst in range(2))
                ops = _pass_weights(p, q)
                for n, op in enumerate(ops):
                    aqkv[j, n, _rows(r, 16), :] = op
                yield ops[8:16]
                yield ops[16:]

        def turn_ffn_in(j, w, release):
            for g in range(F2 // 128):
                for b in range(4):
                    for kind in range(3):
                        n = RG if kind == 2 else 128
                        fT[j, g, kind, b, _rows(0, n), :] = transposed(w, kind, b % 2, 128 * g + b // 2 * F2, n, release)
                    yield []

        def prep_ffn_in(j, src):
            for g in range(F2 // 128):
                for r in range(0, RG, 16):
                    q, p = ([[fT[src, g, kind, b, _rows(RG * inst + r, 16), :] for b in range(4)]
                             for kind in (0, 2 - inst)] for inst in range(2))
                    ops = _pass_weights(p, q)
                    for n, op in enumerate(ops):
                        a13[g, j, n, _rows(r, 16), :] = op
                    for n in range(8, NU, 6):
                        yield ops[n:n + 6]

        def prep_ffn_out():
            for r in range(0, D2, 16):
                for c0 in range(0, F2, 256):
                    n = min(256, F2 - c0)
                    ops = _lhs_operands(
                        *(_pack(w2T[pl.ds(p, 16), pl.ds(c + c0, n)]) for p in (r, D2 + r) for c in (0, F2)))
                    for i in range(7):
                        a2[i, _rows(r, 16), pl.ds(c0, n)] = ops[i]
                    yield tiles(*(ops[i] for i in (0, 1, 4, 5, 6)))

        class Pacer:
            def __init__(self, never):
                self.never, self.slot, self.count, self.jobs, self.recent = never, 0, 0, [], None

            def add(self, gen, steps, first, last):
                self.jobs.append([gen, steps, int(first), int(last), 0])

            def release(self, k):
                return jnp.where(self.never[:, :k.shape[1]], self.recent[:, :k.shape[1]], k)

            def deadline(self):
                deps = []
                self.slot += 1
                for job in self.jobs:
                    gen, steps, first, last, _ = job
                    while job[4] < min(steps, (self.slot - first) * steps // (last + 1 - first)):
                        got = next(gen, [])
                        if gen.__name__[-2:] in tied2:
                            deps += [pltpu.bitcast(x, u32) for x in got]
                        job[4] += 1
                while len(deps) > 1:
                    deps = deps[2:] + [deps[0] | deps[1]]
                return deps

            def dot(self, a, b):
                a = tie(a, self.deadline, [self.never]) if self.count % 4 == pu else _unpack(a)
                out = _dot(a, b)
                self.recent = out[:8]
                self.count += 1
                return out

            def drain(self):
                for job in self.jobs:
                    for _ in job[0]:
                        pass

        M = 49

        def prologue():
            groups = [[x_copy(2), x_copy(3), x_copy(4), w_copy(1)],
                      [x_copy(5), x_copy(6), x_copy(7), w_copy(2), w_copy(3)],
                      [w_copy(4)]]
            x_copy(0).start()
            w_copy(0).start()
            x_copy(0).wait()
            x_copy(1).start()
            corner = xT[0, pl.ds(0, 16), pl.ds(0, 128)].astype(f32)[:8]
            zr = jnp.max(jnp.where(corner * corner < -2.0, 1, 0))
            zr, zf = (zr if x in opq else 0 for x in 'xf')
            for _ in normalize(0):
                pass
            w_copy(0).wait()
            x_copy(1).wait()
            for cp in groups[0]:
                cp.start()
            for _ in prep_qkv(0, None):
                pass
            pace = Pacer(corner * corner < -1.0)
            pace.add(prep_qkv(1, pace.release), 18, 7, M - xl)
            pace.add(prep_qkv(2, pace.release), 18, M - 14, 2 * M - xl - 10)
            pace.add(normalize(1), 38, 2 * M - 14, 3 * M - 8)
            r2, r3, r4 = (M * (x + 1) + 2 for x in waits)
            if not noprol:
                for t, first, last in ((2, r2, 6 * M - 8), (3, 6 * M, 9 * M - 8), (4, 9 * M, r3 - 18),
                                       (5, r3, 15 * M - 8), (6, 15 * M, r4 - 18), (7, r4, 21 * M - 8)):
                    pace.add(normalize(t), 38, first, last)
                pace.add(prep_ffn_out(), 56, 6 * M, r3 - 14)
                pace.add(turn_ffn_in(0, w1, pace.release), 28, r3, r3 + tl * M)
                pace.add(prep_ffn_in(0, zf + 0), 84, r3 + tl * M + 20, r4 + tl * M)
                pace.add(turn_ffn_in(1, w3, pace.release), 28, r4, r4 + tl * M)
                pace.add(prep_ffn_in(1, zf + 1), 84, r4 + tl * M + 20, 24 * M - 8)
                pace.add(prep_square(3, pace.release), 26 + xl, r3 + tl * M, r4 - 10)
                pace.add(spread_keys(0, 0, 0, pace.release), VT * 4 * DH // KG, 3 * M, max(3 * VT + 2, 20) * M)
            for n in range(3 * (1 if noprol else NT)):
                t, j = divmod(n, 3)
                if t == NT - 1:
                    j = (j + 1) % 3

                def event():
                    if n in starts:
                        for cp in groups[1 + starts.index(n)]:
                            cp.start()
                    if n in waits:
                        for cp in groups[waits.index(n)]:
                            cp.wait()

                project(pace, t, t + zr, j, event)
            pace.drain()

        with scope("prologue"):
            prologue()

        NS = 2 * NT
        up = [("g", g, j, n) for g in range(F2 // 128) for shared in (False, True) for j in range(2)
              for n in range(NU) if (PASSES[n][0] in SHARED) == shared]
        down = [("d", i, r, k) for i in ORDER for r in (0, D4) for k in range(F2 // 128)]
        fours = [(up + down)[n:n + 4] for n in range(0, len(up) + len(down), 4)]
        nup = -(-len(up) // 4)
        marks = [nup * (n + 1) // gsteps for n in range(gsteps)]
        marks += [nup + (len(fours) - tailg - nup) * (n + 1) // (NS - gsteps) for n in range(NS - gsteps)]
        program, left = [], list(fours)
        for n in range(NS + 1):
            for c in range(NT):
                if n < NS:
                    program.append([("q", n, c)])
                elif len(left) > (NT - 1 - c) * tailg // NT + 1:
                    program.append(left.pop(0))
                if n > 0:
                    program.append([("v", n - 1, c)])
                if n < gsteps and c in mid:
                    program.append(left.pop(0))
            while n < NS and len(fours) - len(left) < marks[n]:
                program.append(left.pop(0))
        program += left

        def slots(op):
            if op[0] == "q":
                return [wq if op[1] else wq0] * ((TH - (VR if op[2] < VT else 0)) // 16)
            return {"v": [wv] * 2, "g": [wg] * (RG // 16), "d": [wd] * (D4 // 16)}[op[0]]

        weights, due = [], {}
        ends = {}
        for op, *more in program:
            for x in [op] + more:
                if x[0] == "g":
                    ends[x[1]] = len(weights) + RG // 16
                elif x[0] == "d" and x[3] == F2 // 128 - 1:
                    ends.setdefault(F2 // 128, len(weights) - 8 - hlag)
            if op[0] == "v" and op[2] == 0:
                due[op[1]] = len(weights) - slack
            weights += slots(op)
        act = {ends[g] + hlag + (ends[g + 1] - ends[g]) * r // 16: g for g in range(F2 // 128) for r in range(16)}
        for slot in act:
            for back in range(4):
                weights[slot - back] -= wact
        per_step = VT * (2 * VR // (8 * KB)) * DH
        need, pos, have = [], 0, 0
        while have < NS * per_step:
            rate, n = max((((m + 1) * per_step - have) / sum(weights[pos:due[m]]), m) for m in range(NS)
                          if (m + 1) * per_step > have)
            acc = 0
            for w in weights[pos:due[n]]:
                acc += w
                need.append(have + int(acc * rate + 1e-6))
            pos, have = due[n], (n + 1) * per_step
        need += [have] * (len(weights) - len(need))
        switch = sum(x < NT * per_step for x in need)
        nk = VT * 4 * DH // KG if spread else 0
        key_need = [min(nk, (i + 1) * nk // (switch - 60)) for i in range(switch + 10)]
        rest = len(weights) - len(key_need)
        key_need += [nk + min(nk, (i + 1) * nk // (rest - 60)) for i in range(rest)]

        def pair(p, carry):
            sbuf = (s0, s1)
            wsl = p % 2
            rsl = 1 - (p + 1) % 2
            never = [lax.broadcasted_iota(jnp.int32, (8, 128), 0) < -p - k for k in range(ntie + 1)]
            later = {}
            mx = [None] * NS

            def track(n, s):
                mx[n] = s if mx[n] is None else jnp.maximum(mx[n], s)

            def vector_scores():
                for n in range(NS):
                    e, t = divmod(n, NT)
                    for c in range(VT):
                        for r0 in range(0, 2 * VR, 8 * KB):
                            a = [[None, None] for _ in range(KB)]
                            for d in range(DH):
                                qb = [jnp.broadcast_to(qf[p, t, pl.ds(DH * e + d, 1), pl.ds(TH * u, TH)], (8, TH))
                                      for u in range(2)]
                                for k in range(KB):
                                    kv = (kb0, kb1)[e][rsl, c, d, pl.ds(r0 + 8 * k, 8), :]
                                    for u in range(2):
                                        a[k][u] = kv * qb[u] if a[k][u] is None else a[k][u] + kv * qb[u]
                                if d == DH - 1:
                                    for k in range(KB):
                                        s = jnp.concatenate(a[k], 1)
                                        sv[(wsl if insv else 0), n, c, pl.ds(r0 + 8 * k, 8), :] = s
                                        track(n, s)
                                yield [x for row in a for x in row]

            def release(k):
                return jnp.where(never[0], state["recent"], k) if "recent" in state else k

            def next_keys():
                yield from spread_keys(p, 1, wsl, release)
                yield from spread_keys(jnp.minimum(p + 1, NP - 1), 0, 1 - wsl, release)

            side, keys = vector_scores(), next_keys()
            state = dict(slot=0, done=0, tie=0, keys=0)

            def deadline(ntie=ntie):
                slot = state["slot"]
                state["slot"] += 1
                while state["keys"] < key_need[slot]:
                    next(keys)
                    state["keys"] += 1
                last = None
                if slot % every == 0 or slot + 1 in due.values():
                    while state["done"] < need[slot]:
                        last = next(side)
                        state["done"] += 1
                deps = next(pieces) if slot in act else []
                while len(deps) > 1:
                    deps = deps[2:] + [jnp.maximum(deps[0], deps[1])]
                if last is None:
                    return deps
                state["tie"] += ntie
                return deps + [last[(state["tie"] + e) % len(last)] for e in range(ntie)]

            def matmul(a, b, unit=None):
                if unit == 0:
                    state["shared"] = [deadline(4 if four else ntie) for _ in range(a.shape[0] // 8)]
                if unit is None:
                    out = _dot(tie(a, deadline, never), b)
                else:
                    mine = iter([deps[unit::4] if four else deps * (unit == tu) for deps in state["shared"]])
                    out = _dot(tie(a, lambda: next(mine, []), never), b)
                if a.shape[0] > HP // 2:
                    state["recent"] = out[:8, :128]
                return out

            def q_weights(n):
                e, t = divmod(n, NT)
                lo, d0 = _head_window(e)
                win = qf[p, t, pl.ds(lo, HP), :]
                win = jnp.where((row32 >= d0) & (row32 < d0 + DH), win, 0.0)
                parts = [win, jnp.zeros((64 - lo - HP, TQ), f32)]
                half = jnp.concatenate(([jnp.zeros((lo, TQ), f32)] if lo else []) + parts, 0).astype(bf16)
                zero = jnp.zeros((64, TQ), bf16)
                return jnp.concatenate([jnp.concatenate([half, zero], 0), jnp.concatenate([zero, half], 0)], 1)

            def scores(n, c, qw):
                lo = VR if c < VT else 0
                k = kk[p, c, _rows(lo, TH - lo), :]
                s = []
                for x in range(4):
                    depth = 64 * (x // 2) + HP * (n // NT + 1) if short else 128
                    lhs = tie(k, deadline, never) if x == qunit else _unpack(k)
                    s.append(_dot(lhs[:, :depth], qw[:depth, 128 * x:128 * (x + 1)]))
                s = jnp.concatenate(s, 1)
                state["recent"] = s[:8, :128]
                for u in range(2):
                    su = s[:, u * TQ:(u + 1) * TQ]
                    sbuf[n % 2][wsl, c, u, pl.ds(lo, TH - lo), :] = su
                    track(n, jnp.max(su.reshape((TH - lo) // 8, 8, TQ), axis=0))

            def values(n, c, m):
                lo = VR if c < VT else 0
                parts = []
                for u in range(2):
                    if lo:
                        parts.append(sv[(rsl if insv == 1 else wsl if insv else 0), n, c, pl.ds(u * VR, VR), :])
                    parts.append(sbuf[n % 2][rsl, c, u, pl.ds(lo, TH - lo), :])
                pr = jnp.exp2(jnp.concatenate(parts, 0) - m).astype(bf16)
                return matmul(vT[2 * p + n // NT, :, pl.ds(c * TQ, TQ)], pr)

            def finish(n, acc):
                e, t = divmod(n, NT)
                lrow = 0 if e else DH
                oF[p, t, e] = acc * (1.0 / acc[lrow:lrow + 1])

            hidden = []

            def activation():
                for g in range(F2 // 128):
                    parts = []
                    for inst in (1, 0):
                        for r in range(0, RG, 8):
                            gate, up = (_combine([(m0, m1)[g % 2][rsl, j, inst, i, pl.ds(r, 8), :] for i in range(7)])
                                        for j in range(2))
                            ops = _rhs_operands(*((a * b) * jnp.tanh(0.5 * a) + a * b for a, b in zip(gate, up)))
                            if hmem:
                                for i in range(7):
                                    hB[wsl, g, i, pl.ds(8 * len(parts), 8), :] = ops[i]
                            parts.append(ops)
                            if len(parts) == 16:
                                hidden.append([jnp.concatenate(x, 0).astype(bf16) for x in zip(*parts)])
                            yield [ops[i] for i in htie]

            pieces = activation()
            y, res, count = {}, [], 0
            for ops in program:
                for x, op in enumerate(ops):
                    if op[0] == "q":
                        _, n, c = op
                        if c == 0:
                            qw = q_weights(n)
                        scores(n, c, qw)
                    elif op[0] == "v":
                        _, n, c = op
                        if c == 0:
                            assert state["done"] >= (n + 1) * per_step
                            m = jnp.max(mx[n], axis=0, keepdims=True)
                        o = values(n, c, m)
                        acc = o + acc if c else o
                        if c == NT - 1:
                            finish(n, acc)
                    elif op[0] == "g":
                        _, g, j, n = op
                        res.append(matmul(a13[g, j, n], operand(xB.at[p], n), x))
                        res = stage((m0, m1)[g % 2].at[wsl, j], n, res)
                    else:
                        _, i, r, k = op
                        o = matmul(a2[i, _rows(r, D4), pl.ds(128 * k, 128)], hB[rsl if hmem == 1 else wsl, k, i].astype(bf16) if hmem else hidden[k][i], x)
                        y[r, i] = o + y[r, i] if k else o
                        if k == 6 and ymem and i not in ORDER[-2:]:
                            yb[wsl, i, pl.ds(r, D4), :] = y[r, i]
            c = [_combine({i: yb[rsl, i, pl.ds(r, D4), :] if ymem and i not in ORDER[-2:] else y[r, i] for i in ORDER}) for r in (0, D4)]
            yacc[p] = xT[p].astype(f32) + 0.5 * _assemble([c[0][:2], c[1][:2], c[0][2:], c[1][2:]])
            return carry

        with scope("main"):
            if nomain:
                def touch(i, c):
                    r = pl.ds(pl.multiple_of(8 * i, 8), 8)
                    oF[i, 0, 0, r, 0:128] = pltpu.bitcast(
                        a13[i, 0, 0, r, 0:128] | a2[i, r, 0:128] | xB[i, 0, r, :] | kk[i, 0, r, :] | vT[i, r, 0:128], f32
                    ) + qf[i, 0, r, 0:128] + kb0[i, 0, 0, r, :]
                    return c
                lax.fori_loop(0, 2, touch, 0)
            else:
                lax.fori_loop(0, NP, pair, 0)

        def out_copy(t):
            return pltpu.make_async_copy(outb.at[t], outT_hbm.at[:, pl.ds(t * TQ, TQ)], o_sem.at[t])

        def merged(t):
            row8 = lax.broadcasted_iota(jnp.int32, (8, TQ), 0)
            rows = []
            for p in range(NP):
                a, b = oF[p, t, 0], oF[p, t, 1]
                rows += [a[:24], jnp.where(row8 < HP - DH, a[24:], b[:8]), b[8:]]
            o = jnp.concatenate(rows, 0)
            ops = _rhs_operands(*(o[v:v + KH, u:u + TH] for v in (0, KH) for u in (0, TH)))

            def rhs(n):
                i, pieces = PASSES[n]
                return jnp.concatenate(
                    [ops[i][64 * k:64 * k + 64] if k < 3 else o[2 * KH:, TH * REMAINDER[i]:TH * (REMAINDER[i] + 1)]
                     for k in pieces], 0).astype(bf16)
            return rhs

        with scope("tail"):
            for t in range(NT if not noprol else 1):
                rhs = merged(t)
                res = [_dot(_unpack(aqkv[3, n]), rhs(n)) for n in range(NU)]
                outb[t] = (_assemble(_collect(res)) + yacc[t]).astype(bf16)
                out_copy(t).start()
        for t in range(NT):
            out_copy(t).wait()

    return kernel


def build(**kw):
    flags = kw.pop("flags", None)
    name = kw.pop("name", "fused_block")
    VT = max(kw.get("VT", 6), 1)

    def run(A_x, A_wqkv, A_wo, B_x, B_w1, B_w3, B_w2):
        del B_x
        hbm = pl.BlockSpec(memory_space=pltpu.HBM)
        vm = pltpu.VMEM

        def packed(*shape):
            return vm(shape[:-2] + (shape[-2] // 2, shape[-1]), u32)

        outT = pl.pallas_call(
            make_kernel(**kw),
            out_shape=jax.ShapeDtypeStruct((D, S), bf16),
            in_specs=[hbm] * 6,
            out_specs=hbm,
            scratch_shapes=[
                vm((NT, D, TQ), bf16), vm((D, 3 * D), bf16), vm((D, D), bf16),
                vm((D, F), bf16), vm((D, F), bf16), vm((D, F), bf16),
                packed(4, 3, 2, 512, 128), packed(2, 7, 3, 4, 128, 128), packed(4, NU, D4, 128), packed(F2 // 128, 2, NU, RG, 128),
                packed(8, D2, F2),
                packed(NT, 10, KH, TH), vm((NP, NT, 64, TQ), f32), packed(NP, NT, TH, 128),
                vm((2, VT, DH, 32, 128), f32), vm((2, VT, DH, 32, 128), f32),
                packed(H, HP, S), vm((NP, NT, 2, HP, TQ), f32),
                vm((2, NT, 2, TH, TQ), f32), vm((2, NT, 2, TH, TQ), f32), vm((2, 2 * NT, VT, 32, TQ), f32),
                vm((2, 2, 2, 7, RG, TH), f32), vm((2, 2, 2, 7, RG, TH), f32), vm((2, 7, D2, TH), f32), vm((2, 7, 7, 128, TH), f32),
                vm((NT, D, TQ), f32), vm((NT, D, TQ), bf16),
                pltpu.SemaphoreType.DMA((NT,)), pltpu.SemaphoreType.DMA((5,)),
                pltpu.SemaphoreType.DMA((NT,)),
            ],
            compiler_params=pltpu.CompilerParams(vmem_limit_bytes=110 * 2**20, flags=flags),
            name=name,
        )(A_x[0].T, A_wqkv, A_wo, B_w1, B_w3, B_w2.T)
        return outT.T[None]

    return jax.jit(run, keep_unused=True)


_run = build()


@jax.jit
def pallas_parallel_sum__softmax_full_mha__glu_gated_swiglu__prompt_kernel(
    A_x, A_wqkv, A_wo, B_x, B_w1, B_w3, B_w2
):
    return _run(A_x, A_wqkv, A_wo, B_x, B_w1, B_w3, B_w2)
```

```python
import math

import jax
import jax.numpy as jnp
from jax import lax
from jax.experimental import pallas as pl
from jax.experimental.pallas import tpu as pltpu

S, D, H, F = 2048, 448, 16, 1792
DH = D // H
HP = 32
TQ, TH = 256, 128
NT = S // TQ
NP = H // 2
D2, D4, F2 = D // 2, D // 4, F // 2
NG = F2 // 128
KH = 192
VK, VB = 112, 32
EPS = 1e-5
QSCALE = DH ** -0.5 * math.log2(math.e)

f32, bf16, u32 = jnp.float32, jnp.bfloat16, jnp.uint32

REMAINDER = {2: 1, 3: 0, 5: 1, 6: 0}
PASSES = [(i, k) for i in REMAINDER for k in ((0, 1), (2, 3), (0, 1), (2, 3))]
PASSES += [(i, k) for i in (4, 1, 0) for k in ((0, 1), (0, 2), (2, 1))]
NU = len(PASSES)

ROOM_SCORES, ROOM_VALUES = [40, 40, 48, 48, 48, 48, 28, 28], [28, 20]
ROOM_FIRST, ROOM_LAST, ROOM_UP, ROOM_DOWN, ROOM_END, ROOM_ACT = 58, 38, 54, 49, 40, 44
SLACK, ACT_LAG, ACT_END, KEY_END, KEY_LAG, UP_EXTRA, TIES = 20, 10, 20, (45, 40), 2, 2, 3
OUT_SPLIT, TURN_LAG, TURN_SPLIT, TURN_END = 28, 22, 125, 25
FIRST_KEYS, FIRST_SCORES = (5.2, 12.5), (14.2, 23.9)


def _dot(a, b):
    return jnp.dot(a, b, preferred_element_type=f32)


def _pack(x):
    return pltpu.bitcast(x.astype(bf16), u32)


def _unpack(x):
    return pltpu.bitcast(x, bf16)


def _rows(start, n):
    return pl.ds(start // 2, n // 2)


def _cat(parts, axis=0):
    return jnp.concatenate(list(parts), axis)


def _tiles(*xs):
    return [x[r:r + 8, c:c + 128] for x in xs for r in range(0, x.shape[0], 8) for c in range(0, x.shape[1], 128)]


def _lhs_operands(a11, a12, a21, a22):
    return [a11 + a22, a21 + a22, a11, a22, a11 + a12, a21 - a11, a12 - a22]


def _rhs_operands(b11, b12, b21, b22):
    return [b11 + b22, b11, b12 - b22, b21 - b11, b22, b11 + b12, b21 + b22]


def _combine(m):
    m1, m2, m3, m4, m5, m6, m7 = (m[i] for i in range(7))
    return m7 + (m1 + (m4 - m5)), m3 + m5, m4 + m2, m6 + (m1 + (m3 - m2))


def _share(first, third):
    low = lax.broadcasted_iota(jnp.int32, first[0].shape, 1) < 64
    both = jnp.where(low, first[1], first[0])
    diff = _pack(_unpack(jnp.where(low, first[0], first[1])).astype(f32) - _unpack(both).astype(f32))
    return [both, jnp.where(low, diff, third[0]), jnp.where(low, third[1], diff)]


def _finished(n, results):
    i = PASSES[n][0]
    if i in REMAINDER:
        done = [(len(results) // 2 - 1, i, results[-1] + results[-2])] if len(results) % 2 == 0 else []
    else:
        done = [(len(results) - 2, i, results[-1] + results[0])] if len(results) > 1 else []
    if len(results) == (4 if i in REMAINDER else 3):
        results.clear()
    return done


def _after(x, deadline, never, dtype):
    x = pltpu.bitcast(x, dtype)
    rows = []
    for r in range(0, x.shape[0], 8):
        first = x[r:r + 8, :128]
        for mask, dep in zip(never, deadline()):
            first = lax.select(mask, dep, first)
        rows.append(first)
    rows = _cat(rows)
    return _unpack(rows if x.shape[1] == 128 else _cat([rows, x[:, 128:]], 1))


def _first(work, n):
    for _ in range(n):
        yield next(work)


def _delayed(works, lag):
    queue = [[]] * lag
    for work in works:
        for deps in work:
            queue.append(deps)
            yield queue.pop(0)
    yield from queue


class _Pacer:
    def __init__(self, never):
        self.never, self.slot, self.count, self.jobs, self.recent = never, 0, 0, [], None

    def add(self, work, steps, first, last):
        self.jobs.append([work, steps, int(first), int(last), 0])

    def release(self, x):
        n = x.shape[1]
        first = jnp.where(self.never[:, :n], self.recent[:, :n], x[:8])
        return first if x.shape[0] == 8 else _cat([first, x[8:]])

    def deadline(self):
        deps = []
        self.slot += 1
        for job in self.jobs:
            work, steps, first, last, _ = job
            while job[4] < min(steps, (self.slot - first) * steps // (last + 1 - first)):
                deps += [pltpu.bitcast(x, u32) for x in next(work)]
                job[4] += 1
        while len(deps) > 1:
            deps = deps[2:] + [deps[0] | deps[1]]
        return deps

    def dot(self, a, b):
        a = _after(a, self.deadline, [self.never], u32) if self.count % 4 == 0 else _unpack(a)
        out = _dot(a, b)
        self.recent = out[:8]
        self.count += 1
        return out


def _cut(t):
    return VK + 16 * (t * ((S // 2 - VK) // 16) // NT)


def _plan():
    steps, up_steps = 2 * NT, 12
    up = [("up", g, j, n) for g in range(NG) for shared in (False, True) for j in range(2)
          for n in range(NU) if (PASSES[n][0] not in REMAINDER) == shared]
    down = [("down", i, r, k) for i in (2, 3, 4, 1, 0, 6, 5) for r in (0, D4) for k in range(NG)]
    fours = [(up + down)[n:n + 4] for n in range(0, len(up) + len(down), 4)]
    ups = -(-len(up) // 4)
    marks = [UP_EXTRA + (ups - UP_EXTRA) * (n + 1) // up_steps for n in range(up_steps)]
    marks += [ups + (len(fours) - NT - ups) * (n + 1) // (steps - up_steps) for n in range(steps - up_steps)]
    program, left = [], list(fours)
    for n in range(steps + 1):
        for t in range(NT):
            program.append([("scores", n, t)] if n < steps else left.pop(0))
            if n > 0:
                program.append([("values", n - 1, t)])
        while n < steps and len(fours) - len(left) < marks[n]:
            program.append(left.pop(0))
    assert not left

    room, due, ends, calm = [], [], {}, []
    for ops in program:
        for op in ops:
            if op[0] == "up":
                ends[op[1]] = len(room) + 4
            elif op[0] == "down" and op[3] == NG - 1:
                ends.setdefault(NG, len(room) - ACT_END - ACT_LAG)
        kind, n, t = ops[0][:3]
        if kind == "values" and t == 0 and n > 0:
            due.append(len(room) - SLACK)
        if kind == "scores":
            count = (_cut(t + 1) - _cut(t)) // 16
            calm.append(len(room) + count - 4)
            room += [ROOM_FIRST] * count if n == 0 else [ROOM_LAST] * count if t == NT - 1 else ROOM_SCORES[-count:]
        else:
            if kind == "down":
                calm += [len(room) + x for x in (1, 3, 5)]
            room += {"values": ROOM_VALUES, "up": [ROOM_UP] * 4, "down": [ROOM_DOWN] * (D4 // 16)}[kind]
    room[due[-1]:] = [ROOM_END] * (len(room) - due[-1])
    due.append(len(room) - 4)

    activate = []
    for g in range(NG):
        spots = [x for x in calm if ends[g] <= x - ACT_LAG < ends[g + 1]]
        if len(spots) < 16:
            spots = range(ends[g] + ACT_LAG, ends[g + 1] + ACT_LAG)
        activate += [spots[len(spots) * r // 16] for r in range(16)]
    for slot in activate:
        for back in range(4):
            room[slot - back] -= ROOM_ACT // 4

    per_step = 2 * VK // VB * DH
    scores, done = [], 0
    while done < steps * per_step:
        rate, n = max((((m + 1) * per_step - done) / sum(room[len(scores):due[m]]), m) for m in range(steps)
                      if (m + 1) * per_step > done)
        total = 0
        for w in room[len(scores):due[n]]:
            total += w
            scores.append(done + int(total * rate + 1e-6))
        done = (n + 1) * per_step
    scores += [done] * (len(room) - len(scores))

    first, second = (sum(x < n * per_step for x in scores) for n in (NT - 1, steps - 1))
    count = 2 * DH + KEY_LAG
    keys = [min(count, (i + 1) * count // (first - KEY_END[0])) for i in range(first + 10)]
    keys += [count + min(count, (i + 1) * count // (second - first - KEY_END[1]))
             for i in range(len(room) - len(keys))]
    return program, scores, keys, activate


def _kernel(xT_hbm, wqkv_hbm, wo_hbm, w1_hbm, w3_hbm, w2T_hbm, outT_hbm,
            xT, wqkv, wo, w1, w3, w2T, a_qkv, a_up, a_down, a_o0, a_o1,
            xB, qf, kf, kk, kb0, kb1, vT, s0, s1, sv, sv0, mB, hB, oF, y, outb, sems):
    row32 = lax.broadcasted_iota(jnp.int32, (HP, TQ), 0)

    def window(e):
        return (2 * DH - HP, row32 >= HP - DH) if e else (0, row32 < DH)

    def normalize(t):
        acc = 0.0
        for r in range(0, D, 64):
            acc = acc + jnp.sum(xT[t, pl.ds(r, 64), :].astype(f32).reshape(8, 8, TQ), axis=0)
            yield _tiles(acc)
        mean = jnp.sum(acc, axis=0, keepdims=True) * (1.0 / D)
        acc = 0.0
        for r in range(0, D, 32):
            xc = xT[t, pl.ds(r, 32), :].astype(f32) - mean
            acc = acc + jnp.sum((xc * xc).reshape(4, 8, TQ), axis=0)
            yield _tiles(acc)
        scale = lax.rsqrt(jnp.sum(acc, axis=0, keepdims=True) * (1.0 / D) + EPS)
        yield []

        def block(r):
            x = (xT[t, pl.ds(r, 16), :].astype(f32) - mean) * scale
            return [x[:, :TH], x[:, TH:]]

        for r in range(0, KH, 16):
            b = block(r) + block(KH + r)
            words = _pack(_cat(_rhs_operands(*b) + b[1:3], 1))
            for i in range(9):
                xB[t, i, _rows(r, 16), :] = words[:, i * TH:(i + 1) * TH]
            yield _tiles(words)[:4]
            yield _tiles(words)[4:]
        for r in range(0, 64, 16):
            words = _pack(_cat(block(2 * KH + r), 1))
            for u in range(2):
                xB[t, 9, _rows(64 * u + r, 16), :] = words[:, u * TH:(u + 1) * TH]
            yield _tiles(words)

    def pass_weights(dst, w, release):
        def turned(i, *pieces):
            starts = [(64 * k, KH + 64 * k) if k < 3 else (2 * KH, 2 * KH) for k in pieces]
            blk = _cat(_lhs_operands(*(w(r, m) for m in range(2) for r in rows))[i] for rows in starts)
            words = _pack(release(blk).astype(bf16).T)
            return words[:len(words) // 2], words[len(words) // 2:]

        n = 0
        while n < NU:
            i = PASSES[n][0]
            first = turned(i, 0, 1)
            yield [first[1][-8:]]
            if i in REMAINDER:
                second = turned(i, 2, 3)
                ops = [first[0], second[0], first[1], second[1]]
            else:
                ops = _share(first, turned(i, 2, 2))
            for op in ops:
                dst[n] = op
                n += 1
            yield [ops[-1][-8:]]

    def prepare_qkv(j, release=None):
        skew = j * D % 128
        parts = [[], [], [], []]
        for col in range(j * D - skew, j * D - skew + D, 128):
            n = min(128, 3 * D - col)
            for part, starts in zip(parts, ((0, 64), (128, 128), (192, 256), (320, 384))):
                blk = _cat(wqkv[pl.ds(r, 64), pl.ds(col, n)] for r in starts)
                if release is not None:
                    blk = pltpu.bitcast(release(pltpu.bitcast(blk, f32)), bf16)
                part.append(_pack(blk.T))
                yield []
        for m in range(2):
            a, b, c, e = ([_cat(part)[(skew + r) // 2:(skew + r + D4) // 2] for r in (m * D2, m * D2 + D4)]
                          for part in parts)
            both, own0, own1 = _share(a, b)
            for n, op in enumerate((c[0], e[0], both, own0, c[1], e[1], own1)):
                a_qkv[j, 7 * m + n] = op
            yield []

    def prepare_up(j, w, release):
        for g in range(NG):
            def piece(r, m):
                x = w[pl.ds(r, 64), pl.ds(m * F2 + 128 * g, 128)].astype(f32)
                return x if j else 0.5 * x
            yield from pass_weights(a_up.at[g, j], piece, release)

    def prepare_o(release):
        shifted = []
        for r in range(0, D, 64):
            blk = wo[pl.ds(r, 64), pl.ds(256, D - 256)].astype(f32)
            shifted.append(_cat([release(blk[:, :128]), blk[:, 128:]], 1)[:, 96:])
            yield []
        yield from pass_weights(a_o0, lambda r, m: wo[pl.ds(r, 64), pl.ds(128 * m, 128)].astype(f32), release)
        yield from pass_weights(
            a_o1, lambda r, m: shifted[r // 64] if m else wo[pl.ds(r, 64), pl.ds(256, 96)].astype(f32), release)

    def prepare_down():
        for r in range(0, D2, 16):
            for col in range(0, F2, 256):
                n = min(256, F2 - col)
                a = [w2T[pl.ds(row, 16), pl.ds(half + col, n)]
                     for row in ((r, r + 128) if r < 128 else (r + 128, r + D2)) for half in (0, F2)]
                ops = _lhs_operands(*(x.astype(f32) for x in a))
                ops = [_pack(x) for x in ops[:2] + [a[0], a[3]] + ops[4:]]
                for i in range(7):
                    a_down[i, _rows(r, 16), pl.ds(col, n)] = ops[i]
                yield _tiles(*ops[:2], *ops[4:])

    def spread_keys(p, e, slot, release):
        for u in range(2):
            for d in range(DH):
                row = release(jnp.broadcast_to(kf[p, pl.ds(DH * e + d, 1), pl.ds(u * TH, TH)], (8, TH)))
                col = _cat([row[:, :VK]] * 16).T
                (kb0, kb1)[e][slot, d, pl.ds(u * VK, VK), :] = col
                yield [col[-8:]]

    def vector_scores(p, n, src, dst, track=None):
        e, t = divmod(n, NT)
        q = [_cat((jnp.broadcast_to(qf[p, t, pl.ds(DH * e + d, 1), pl.ds(col, TH)], (VB, TH))
                   for col in (0, TH)), 1) for d in range(DH)]
        for r in range(0, 2 * VK, VB):
            k = (kb0, kb1)[e][src, :, pl.ds(r, VB), :].reshape(DH * VB, 128)
            k = _cat([k, k], 1)
            for d in range(DH):
                term = k[VB * d:VB * (d + 1)] * q[d]
                s = s + term if d else term
                if d == DH - 1:
                    (sv.at[dst, n] if n else sv0.at[dst])[pl.ds(r, VB), :] = s
                    if track:
                        track(n, s)
                yield s

    def project(pace, t, j, m):
        def rhs(u, *pieces):
            where = ((1, 8), (7, 4))[u]
            return _unpack(_cat(
                xB[t, where[k // 3], _rows(64 * (k % 3), 64), :] if k < 6 else xB[t, 9, _rows(64 * u, 64), :]
                for k in pieces))

        out = []
        for u in range(2):
            r = [pace.dot(a_qkv[j, 7 * m + n], rhs(u, *pieces)) for n, pieces in enumerate(
                ((3, 4), (5, 6), (0, 1), (0, 2), (3, 4), (5, 6), (2, 1)))]
            out += [r[3] + (r[2] + (r[1] + r[0])), r[6] + (r[2] + (r[5] + r[4]))]
        out = _cat([_cat(out[0::2], 1), _cat(out[1::2], 1)])
        for x in range(NP // 2):
            p, blk = NP // 2 * m + x, out[2 * DH * x:2 * DH * (x + 1)]
            if j == 0:
                qf[p, t, pl.ds(0, 2 * DH), :] = blk * QSCALE
            elif j == 1:
                if t == 0:
                    kf[p, pl.ds(0, 2 * DH), :] = blk
                gap = jnp.zeros((8, TH), f32)
                kk[p, _rows(t * TH, TH), :] = _pack(_cat([blk[:, :TH], gap, blk[:, TH:], gap]).astype(bf16).T)
            else:
                for e in range(2):
                    ones = jnp.where(row32 == (0 if e else DH), 1.0, 0.0)
                    lo, inside = window(e)
                    vT[2 * p + e, :, pl.ds(t * TQ, TQ)] = _pack(jnp.where(inside, blk[lo:lo + HP], ones))

    def prologue():
        x = [(xT_hbm.at[:, pl.ds(t * TQ, TQ)], xT.at[t]) for t in range(NT)]
        wq, wkv = ((wqkv_hbm.at[:, cols], wqkv.at[:, cols]) for cols in (pl.ds(0, 512), pl.ds(512, 3 * D - 512)))
        groups = [x[:1], [wq, x[1]], [wkv], x[2:], [(wo_hbm, wo), (w2T_hbm, w2T), (w1_hbm, w1)], [(w3_hbm, w3)]]
        groups = [[pltpu.make_async_copy(src, dst, sems.at[i]) for src, dst in group]
                  for i, group in enumerate(groups)]
        starts, waits = {1: 3, 4: 4, 12: 5}, {1.5: 2, 5: 3, 14: 4, 19: 5}
        for cp in groups[0] + groups[1]:
            cp.start()
        groups[0][0].wait()
        for _ in normalize(0):
            pass
        groups[2][0].start()
        for cp in groups[1]:
            cp.wait()
        for _ in prepare_qkv(0):
            pass

        corner = xT[0, pl.ds(0, 16), pl.ds(0, 128)].astype(f32)[:8]
        pace = _Pacer(corner * corner < -1.0)
        order = [(0, 0), (1, 0), (0, 1), (1, 1), (0, 2), (1, 2)] + [(t, 1) for t in range(2, NT)]
        order += [(t, j) for t in range(2, NT) for j in (2, 0)]
        each = 49
        _, first, third, fourth = (each * n + 4 for n in waits)
        pace.add(normalize(1), 50, 0, each - 6)
        pace.add(prepare_qkv(2, pace.release), 18, 2 * each + 9, 4 * each - 8)
        for t in range(2, NT):
            last = each * order.index((t, 1)) - 6
            pace.add(normalize(t), 50, first, last)
            first = last
        down = prepare_down()
        pace.add(down, OUT_SPLIT, third, fourth - 14)
        pace.add(down, 56 - OUT_SPLIT, fourth, 24 * each - 8)
        out = prepare_o(pace.release)
        turns = _delayed([_first(out, 7), prepare_up(0, w1, pace.release), out, prepare_up(1, w3, pace.release)],
                         TURN_LAG)
        assert TURN_SPLIT <= 35 + 14 * NG
        pace.add(turns, TURN_SPLIT, third, fourth - TURN_END)
        pace.add(turns, 35 + 28 * NG + TURN_LAG - TURN_SPLIT, fourth, 24 * each - 2)
        pace.add(_delayed([spread_keys(0, 0, 0, pace.release)], 6), 2 * DH + 6, *(each * n for n in FIRST_KEYS))
        pace.add(([_tiles(s)[n % (VB // 4)]] for n, s in enumerate(vector_scores(0, 0, 0, 0))),
                 2 * VK // VB * DH, *(each * n for n in FIRST_SCORES))
        for n, (t, j) in enumerate(order):
            for m in range(2):
                project(pace, t, j, m)
                now = n + (m + 1) / 2
                if now in starts:
                    for cp in groups[starts[now]]:
                        cp.start()
                if now in waits:
                    for cp in groups[waits[now]]:
                        cp.wait()
                if waits.get(now) == 2:
                    for _ in prepare_qkv(1):
                        pass
        assert all(job[4] == job[1] for job in pace.jobs)

    program, score_plan, key_plan, activate = _plan()

    def pair(p, carry):
        put, get = p % 2, 1 - (p + 1) % 2
        never = [lax.broadcasted_iota(jnp.int32, (8, 128), 0) < -p - k for k in range(TIES + 2)]
        following = jnp.minimum(p + 1, NP - 1)
        peak = {}
        state = dict(slot=0, scores=0, keys=0, turn=0)

        def track(n, s):
            s = jnp.max(s.reshape(-1, 8, TQ), axis=0)
            peak[n] = jnp.maximum(peak[n], s) if n in peak else s

        def all_vector_scores():
            for n in range(1, 2 * NT):
                yield from vector_scores(p, n, get, put, track)
            yield from vector_scores(following, 0, 1 - get, 1 - put)

        def release(k):
            return lax.select(never[0], state["recent"], k) if "recent" in state else k

        def next_keys():
            yield from _delayed([spread_keys(p, 1, put, release)], KEY_LAG)
            yield from _delayed([spread_keys(following, 0, 1 - put, release)], KEY_LAG)

        def activation():
            for g in range(NG):
                for r in range(0, 128, 8):
                    gate, up = (_combine(mB[put, g, j, :, pl.ds(r, 8), :]) for j in range(2))
                    ops = _rhs_operands(*((a * jnp.tanh(a) + a) * b for a, b in zip(gate, up)))
                    hB[put, g, :, pl.ds(r, 8), :] = jnp.stack(ops)
                    yield ops[6]

        side_scores, side_keys, side_hidden = all_vector_scores(), next_keys(), activation()

        def deadline():
            slot = state["slot"]
            state["slot"] += 1
            deps = [next(side_hidden)] if slot in activate else []
            while state["keys"] < key_plan[slot]:
                deps += next(side_keys)
                state["keys"] += 1
            if state["scores"] < score_plan[slot]:
                while state["scores"] < score_plan[slot]:
                    last = next(side_scores)
                    state["scores"] += 1
                for _ in range(TIES):
                    r, col = divmod(state["turn"] % (VB // 4), 2)
                    deps.append(last[8 * r:8 * r + 8, TH * col:TH * (col + 1)])
                    state["turn"] += 1
            return deps

        def lhs(x, paced):
            return _after(x, deadline, never, f32) if paced else _unpack(x)

        def queries(n):
            e, t = divmod(n, NT)
            lo, inside = window(e)
            win = jnp.where(inside, qf[p, t, pl.ds(lo, HP), :], 0.0)
            after = [jnp.zeros((8, TQ), f32)] * e
            return [_cat([jnp.zeros((64 * u + lo, TQ), f32)] * (u + e > 0) + [win] + after).astype(bf16)
                    for u in range(2)]

        def scores(n, t, q):
            lo, hi = _cut(t), _cut(t + 1)
            k = kk[p, _rows(lo, hi - lo), :]
            for u in range(2):
                s = _cat((_dot(lhs(k, u and x)[:, :q[u].shape[0]], q[u][:, x * TH:(x + 1) * TH])
                          for x in range(2)), 1)
                (s0, s1)[n % 2][put, u, pl.ds(lo, hi - lo), :] = s
                track(n, s)
            state["recent"] = s[:8, :128]

        def values(n, t, m):
            lo, hi = max(t * TH, VK), (t + 1) * TH
            parts = []
            for u in range(2):
                if t == 0:
                    parts.append((sv.at[put, n] if n else sv0.at[get])[pl.ds(u * VK, VK), :])
                parts.append((s0, s1)[n % 2][get, u, pl.ds(lo, hi - lo), :])
            weights = jnp.exp2(_cat(parts) - m).astype(bf16)
            return _dot(lhs(vT[2 * p + n // NT, :, pl.ds(t * TQ, TQ)], True), weights)

        track(0, sv0[put])
        results = []
        for ops in program:
            for unit, op in enumerate(ops):
                if op[0] == "scores":
                    _, n, t = op
                    if t == 0:
                        q = queries(n)
                    scores(n, t, q)
                elif op[0] == "values":
                    _, n, t = op
                    if t == 0:
                        assert state["scores"] >= n * 2 * VK // VB * DH
                        m = jnp.max(peak.pop(n), axis=0, keepdims=True)
                    acc = values(n, t, m) + acc if t else values(n, t, m)
                    if t == NT - 1:
                        total = 0 if n >= NT else DH
                        oF[p, n % NT, n // NT] = acc * (1.0 / acc[total:total + 1])
                elif op[0] == "up":
                    _, g, j, n = op
                    i, pieces = PASSES[n]
                    b = _cat(xB[p, i, _rows(64 * k, 64), :] if k < 3 else xB[p, 9, _rows(64 * REMAINDER[i], 64), :]
                             for k in pieces)
                    results.append(_dot(lhs(a_up[g, j, n], unit == 0), _unpack(b)))
                    state["recent"] = results[-1][:8]
                    for block, i, value in _finished(n, results):
                        mB[put, g, j, i, pl.ds(64 * block, 64), :] = value
                else:
                    _, i, r, k = op
                    part = _dot(lhs(a_down[i, _rows(r, D4), pl.ds(128 * k, 128)], unit == 0),
                                hB[put, k, i].astype(bf16))
                    state["recent"] = part[:8]
                    down = part + down if k else part
                    if k == NG - 1:
                        y[p, i, pl.ds(r, D4), :] = down
        assert not peak and all(next(side, None) is None for side in (side_scores, side_keys, side_hidden))
        return carry

    def epilogue():
        copies = []
        for t in range(NT):
            rows = []
            for p in range(NP):
                a, b = oF[p, t, 0], oF[p, t, 1]
                rows += [a[:HP - 8], jnp.where(row32[:8] < HP - DH, a[HP - 8:], b[:8]), b[8:]]
            o = _cat(rows)
            ops = _rhs_operands(*(o[r:r + KH, col:col + TH] for r in (0, KH) for col in (0, TH)))
            rhs = [_cat(ops[i][64 * k:64 * k + 64] if k < 3 else o[2 * KH:, TH * REMAINDER[i]:TH * (REMAINDER[i] + 1)]
                        for k in pieces).astype(bf16) for i, pieces in PASSES]
            for a_o, first, size in ((a_o0, 0, 64), (a_o1, 128, 48)):
                results, products = [], [{}, {}]
                for n in (*range(8), *range(16, NU), *range(8, 16)):
                    results.append(_dot(_unpack(a_o[n]), rhs[n]))
                    for block, i, value in _finished(n, results):
                        products[block][i] = value + y[t, i, pl.ds(first + block * size, size), :]
                out = [_combine(x) for x in products]
                out = _cat(_cat(out[block][2 * m:2 * m + 2], 1) for m in range(2) for block in range(2))
                span = pl.ds(2 * first, 4 * size)
                outb[t, span, :] = (xT[t, span, :].astype(f32) + out).astype(bf16)
                copies.append(pltpu.make_async_copy(
                    outb.at[t, span], outT_hbm.at[span, pl.ds(t * TQ, TQ)], sems.at[6]))
                copies[-1].start()
        for cp in copies:
            cp.wait()

    prologue()
    lax.fori_loop(0, NP, pair, 0)
    epilogue()


@jax.jit
def pallas_parallel_sum__softmax_full_mha__glu_gated_swiglu__prompt_kernel(
    A_x: jax.Array,
    A_wqkv: jax.Array,
    A_wo: jax.Array,
    B_x: jax.Array,
    B_w1: jax.Array,
    B_w3: jax.Array,
    B_w2: jax.Array,
):
    del B_x
    hbm = pl.BlockSpec(memory_space=pltpu.HBM)
    vm = pltpu.VMEM

    def packed(*shape):
        return vm(shape[:-2] + (shape[-2] // 2, shape[-1]), u32)

    scratch = [
        vm((NT, D, TQ), bf16), vm((D, 3 * D), bf16), vm((D, D), bf16),
        vm((D, F), bf16), vm((D, F), bf16), vm((D, F), bf16),
        packed(3, 16, D4, 128), packed(NG, 2, NU, 64, 128), packed(8, D2, F2),
        packed(NU, 64, 128), packed(NU + 3, 48, 128),
        packed(NT, 10, KH, TH), vm((NP, NT, 64, TQ), f32), vm((NP, 64, TQ), f32),
        packed(NP, S // 2, 128), vm((2, DH, 2 * VK, 128), f32),
        vm((2, DH, 2 * VK, 128), f32), packed(H, HP, S),
        vm((2, 2, S // 2, TQ), f32), vm((2, 2, S // 2, TQ), f32),
        vm((2, 2 * NT, 2 * VK, TQ), f32), vm((2, 2 * VK, TQ), f32),
        vm((2, NG, 2, 7, 128, TH), f32), vm((2, NG, 7, 128, TH), f32),
        vm((NP, NT, 2, HP, TQ), f32), vm((NT, 7, D2, TH), f32), vm((NT, D, TQ), bf16),
        pltpu.SemaphoreType.DMA((7,)),
    ]
    outT = pl.pallas_call(
        _kernel,
        out_shape=jax.ShapeDtypeStruct((D, S), bf16),
        in_specs=[hbm] * 6,
        out_specs=hbm,
        scratch_shapes=scratch,
        compiler_params=pltpu.CompilerParams(vmem_limit_bytes=100 * 2**20),
    )(A_x[0].T, A_wqkv, A_wo, B_w1, B_w3, B_w2.T)
    return outT.T[None]
```

```python
import math

import jax
import jax.numpy as jnp
from jax import lax
from jax.experimental import pallas as pl
from jax.experimental.pallas import tpu as pltpu

S, D, H, F = 2048, 448, 16, 1792
DH = D // H
HP = 32
TQ, TH = 256, 128
NT = S // TQ
NP = H // 2
D2, D4, F2 = D // 2, D // 4, F // 2
NG = F2 // 128
KH = 192
VK, VB = 112, 32
EPS = 1e-5
QSCALE = DH ** -0.5 * math.log2(math.e)

f32, bf16, u32 = jnp.float32, jnp.bfloat16, jnp.uint32

REMAINDER = {2: 1, 3: 0, 5: 1, 6: 0}
PASSES = [(i, k) for i in REMAINDER for k in ((0, 1), (2, 3), (0, 1), (2, 3))]
PASSES += [(i, k) for i in (4, 1, 0) for k in ((0, 1), (0, 2), (2, 1))]
NU = len(PASSES)

ROOM_SCORES, ROOM_VALUES = [40, 40, 48, 48, 48, 48, 28, 28], [28, 20]
ROOM_FIRST, ROOM_LAST, ROOM_UP, ROOM_DOWN, ROOM_END, ROOM_ACT = 58, 38, 54, 49, 40, 44
SLACK, ACT_LAG, ACT_END, KEY_END, KEY_LAG, UP_EXTRA, TIES = 20, 10, 20, (60, 40), 2, 2, 3
OUT_SPLIT, TURN_LAG, TURN_SPLIT, TURN_END = 28, 22, 125, 25
FIRST_KEYS, FIRST_SCORES = (5.2, 12.5), (14.2, 23.9)


def _dot(a, b):
    return jnp.dot(a, b, preferred_element_type=f32)


def _pack(x):
    return pltpu.bitcast(x.astype(bf16), u32)


def _unpack(x):
    return pltpu.bitcast(x, bf16)


def _rows(start, n):
    return pl.ds(start // 2, n // 2)


def _cat(parts, axis=0):
    return jnp.concatenate(list(parts), axis)


def _tiles(*xs):
    return [x[r:r + 8, c:c + 128] for x in xs for r in range(0, x.shape[0], 8) for c in range(0, x.shape[1], 128)]


def _lhs_operands(a11, a12, a21, a22):
    return [a11 + a22, a21 + a22, a11, a22, a11 + a12, a21 - a11, a12 - a22]


def _rhs_operands(b11, b12, b21, b22):
    return [b11 + b22, b11, b12 - b22, b21 - b11, b22, b11 + b12, b21 + b22]


def _combine(m):
    m1, m2, m3, m4, m5, m6, m7 = (m[i] for i in range(7))
    return m7 + (m1 + (m4 - m5)), m3 + m5, m4 + m2, m6 + (m1 + (m3 - m2))


def _share(first, third):
    low = lax.broadcasted_iota(jnp.int32, first[0].shape, 1) < 64
    both = jnp.where(low, first[1], first[0])
    diff = _pack(_unpack(jnp.where(low, first[0], first[1])).astype(f32) - _unpack(both).astype(f32))
    return [both, jnp.where(low, diff, third[0]), jnp.where(low, third[1], diff)]


def _finished(n, results):
    i = PASSES[n][0]
    if i in REMAINDER:
        done = [(len(results) // 2 - 1, i, results[-1] + results[-2])] if len(results) % 2 == 0 else []
    else:
        done = [(len(results) - 2, i, results[-1] + results[0])] if len(results) > 1 else []
    if len(results) == (4 if i in REMAINDER else 3):
        results.clear()
    return done


def _after(x, deadline, never, dtype):
    x = pltpu.bitcast(x, dtype)
    rows = []
    for r in range(0, x.shape[0], 8):
        first = x[r:r + 8, :128]
        for mask, dep in zip(never, deadline()):
            first = lax.select(mask, dep, first)
        rows.append(first)
    rows = _cat(rows)
    return _unpack(rows if x.shape[1] == 128 else _cat([rows, x[:, 128:]], 1))


def _first(work, n):
    for _ in range(n):
        yield next(work)


def _delayed(works, lag):
    queue = [[]] * lag
    for work in works:
        for deps in work:
            queue.append(deps)
            yield queue.pop(0)
    yield from queue


class _Pacer:
    def __init__(self, never):
        self.never, self.slot, self.count, self.jobs, self.recent = never, 0, 0, [], None

    def add(self, work, steps, first, last):
        self.jobs.append([work, steps, int(first), int(last), 0])

    def release(self, x):
        n = x.shape[1]
        first = jnp.where(self.never[:, :n], self.recent[:, :n], x[:8])
        return first if x.shape[0] == 8 else _cat([first, x[8:]])

    def deadline(self):
        deps = []
        self.slot += 1
        for job in self.jobs:
            work, steps, first, last, _ = job
            while job[4] < min(steps, (self.slot - first) * steps // (last + 1 - first)):
                deps += [pltpu.bitcast(x, u32) for x in next(work)]
                job[4] += 1
        while len(deps) > 1:
            deps = deps[2:] + [deps[0] | deps[1]]
        return deps

    def dot(self, a, b):
        a = _after(a, self.deadline, [self.never], u32) if self.count % 4 == 0 else _unpack(a)
        out = _dot(a, b)
        self.recent = out[:8]
        self.count += 1
        return out


def _cut(t):
    return VK + 16 * (t * ((S // 2 - VK) // 16) // NT)


def _plan():
    steps, up_steps = 2 * NT, 12
    up = [("up", g, j, n) for g in range(NG) for shared in (False, True) for j in range(2)
          for n in range(NU) if (PASSES[n][0] not in REMAINDER) == shared]
    down = [("down", i, r, k) for i in (2, 3, 4, 1, 0, 6, 5) for r in (0, D4) for k in range(NG)]
    fours = [(up + down)[n:n + 4] for n in range(0, len(up) + len(down), 4)]
    ups = -(-len(up) // 4)
    marks = [UP_EXTRA + (ups - UP_EXTRA) * (n + 1) // up_steps for n in range(up_steps)]
    marks += [ups + (len(fours) - NT - ups) * (n + 1) // (steps - up_steps) for n in range(steps - up_steps)]
    program, left = [], list(fours)
    for n in range(steps + 1):
        for t in range(NT):
            program.append([("scores", n, t)] if n < steps else left.pop(0))
            if n > 0:
                program.append([("values", n - 1, t)])
        while n < steps and len(fours) - len(left) < marks[n]:
            program.append(left.pop(0))
    assert not left

    room, due, ends, calm = [], [], {}, []
    for ops in program:
        for op in ops:
            if op[0] == "up":
                ends[op[1]] = len(room) + 4
            elif op[0] == "down" and op[3] == NG - 1:
                ends.setdefault(NG, len(room) - ACT_END - ACT_LAG)
        kind, n, t = ops[0][:3]
        if kind == "values" and t == 0 and n > 0:
            due.append(len(room) - SLACK)
        if kind == "scores":
            count = (_cut(t + 1) - _cut(t)) // 16
            calm.append(len(room) + count - 4)
            room += [ROOM_FIRST] * count if n == 0 else [ROOM_LAST] * count if t == NT - 1 else ROOM_SCORES[-count:]
        else:
            if kind == "down":
                calm += [len(room) + x for x in (1, 3, 5)]
            room += {"values": ROOM_VALUES, "up": [ROOM_UP] * 4, "down": [ROOM_DOWN] * (D4 // 16)}[kind]
    room[due[-1]:] = [ROOM_END] * (len(room) - due[-1])
    due.append(len(room) - 4)

    activate = []
    for g in range(NG):
        spots = [x for x in calm if ends[g] <= x - ACT_LAG < ends[g + 1]]
        if len(spots) < 16:
            spots = range(ends[g] + ACT_LAG, ends[g + 1] + ACT_LAG)
        activate += [spots[len(spots) * r // 16] for r in range(16)]
    for slot in activate:
        for back in range(4):
            room[slot - back] -= ROOM_ACT // 4

    per_step = 2 * VK // VB * DH
    scores, done = [], 0
    while done < steps * per_step:
        rate, n = max((((m + 1) * per_step - done) / sum(room[len(scores):due[m]]), m) for m in range(steps)
                      if (m + 1) * per_step > done)
        total = 0
        for w in room[len(scores):due[n]]:
            total += w
            scores.append(done + int(total * rate + 1e-6))
        done = (n + 1) * per_step
    scores += [done] * (len(room) - len(scores))

    first, second = (sum(x < n * per_step for x in scores) for n in (NT - 1, steps - 1))
    count = 2 * DH + KEY_LAG
    keys = [min(count, (i + 1) * count // (first - KEY_END[0])) for i in range(first + 10)]
    keys += [count + min(count, (i + 1) * count // (second - first - KEY_END[1]))
             for i in range(len(room) - len(keys))]
    return program, scores, keys, activate


def _kernel(xT_hbm, wqkv_hbm, wo_hbm, w1_hbm, w3_hbm, w2T_hbm, outT_hbm,
            xT, wqkv, wo, w1, w3, w2T, a_qkv, a_up, a_down, a_o0, a_o1,
            xB, qf, kf, kk, kb0, kb1, vT, s0, s1, sv, sv0, mB, hB, oF, y, outb, sems):
    row32 = lax.broadcasted_iota(jnp.int32, (HP, TQ), 0)

    def window(e):
        return (2 * DH - HP, row32 >= HP - DH) if e else (0, row32 < DH)

    def normalize(t):
        acc = 0.0
        for r in range(0, D, 64):
            acc = acc + jnp.sum(xT[t, pl.ds(r, 64), :].astype(f32).reshape(8, 8, TQ), axis=0)
            yield _tiles(acc)
        mean = jnp.sum(acc, axis=0, keepdims=True) * (1.0 / D)
        acc = 0.0
        for r in range(0, D, 32):
            xc = xT[t, pl.ds(r, 32), :].astype(f32) - mean
            acc = acc + jnp.sum((xc * xc).reshape(4, 8, TQ), axis=0)
            yield _tiles(acc)
        scale = lax.rsqrt(jnp.sum(acc, axis=0, keepdims=True) * (1.0 / D) + EPS)
        yield []

        def block(r):
            x = (xT[t, pl.ds(r, 16), :].astype(f32) - mean) * scale
            return [x[:, :TH], x[:, TH:]]

        for r in range(0, KH, 16):
            b = block(r) + block(KH + r)
            words = _pack(_cat(_rhs_operands(*b) + b[1:3], 1))
            for i in range(9):
                xB[t, i, _rows(r, 16), :] = words[:, i * TH:(i + 1) * TH]
            yield _tiles(words)[:4]
            yield _tiles(words)[4:]
        for r in range(0, 64, 16):
            words = _pack(_cat(block(2 * KH + r), 1))
            for u in range(2):
                xB[t, 9, _rows(64 * u + r, 16), :] = words[:, u * TH:(u + 1) * TH]
            yield _tiles(words)

    def pass_weights(dst, w, release):
        def turned(i, *pieces):
            starts = [(64 * k, KH + 64 * k) if k < 3 else (2 * KH, 2 * KH) for k in pieces]
            blk = _cat(_lhs_operands(*(w(r, m) for m in range(2) for r in rows))[i] for rows in starts)
            words = _pack(release(blk).astype(bf16).T)
            return words[:len(words) // 2], words[len(words) // 2:]

        n = 0
        while n < NU:
            i = PASSES[n][0]
            first = turned(i, 0, 1)
            yield [first[1][-8:]]
            if i in REMAINDER:
                second = turned(i, 2, 3)
                ops = [first[0], second[0], first[1], second[1]]
            else:
                ops = _share(first, turned(i, 2, 2))
            for op in ops:
                dst[n] = op
                n += 1
            yield [ops[-1][-8:]]

    def prepare_qkv(j, release=None):
        skew = j * D % 128
        parts = [[], [], [], []]
        for col in range(j * D - skew, j * D - skew + D, 128):
            n = min(128, 3 * D - col)
            for part, starts in zip(parts, ((0, 64), (128, 128), (192, 256), (320, 384))):
                blk = _cat(wqkv[pl.ds(r, 64), pl.ds(col, n)] for r in starts)
                if release is not None:
                    blk = pltpu.bitcast(release(pltpu.bitcast(blk, f32)), bf16)
                part.append(_pack(blk.T))
                yield []
        for m in range(2):
            a, b, c, e = ([_cat(part)[(skew + r) // 2:(skew + r + D4) // 2] for r in (m * D2, m * D2 + D4)]
                          for part in parts)
            both, own0, own1 = _share(a, b)
            for n, op in enumerate((c[0], e[0], both, own0, c[1], e[1], own1)):
                a_qkv[j, 7 * m + n] = op
            yield []

    def prepare_up(j, w, release):
        for g in range(NG):
            yield from pass_weights(
                a_up.at[g, j], lambda r, m: w[pl.ds(r, 64), pl.ds(m * F2 + 128 * g, 128)].astype(f32), release)

    def prepare_o(release):
        shifted = []
        for r in range(0, D, 64):
            blk = wo[pl.ds(r, 64), pl.ds(256, D - 256)].astype(f32)
            shifted.append(_cat([release(blk[:, :128]), blk[:, 128:]], 1)[:, 96:])
            yield []
        yield from pass_weights(a_o0, lambda r, m: wo[pl.ds(r, 64), pl.ds(128 * m, 128)].astype(f32), release)
        yield from pass_weights(
            a_o1, lambda r, m: shifted[r // 64] if m else wo[pl.ds(r, 64), pl.ds(256, 96)].astype(f32), release)

    def prepare_down():
        for r in range(0, D2, 16):
            for col in range(0, F2, 256):
                n = min(256, F2 - col)
                a = [w2T[pl.ds(row, 16), pl.ds(half + col, n)]
                     for row in ((r, r + 128) if r < 128 else (r + 128, r + D2)) for half in (0, F2)]
                ops = _lhs_operands(*(x.astype(f32) for x in a))
                ops = [_pack(x) for x in ops[:2] + [a[0], a[3]] + ops[4:]]
                for i in range(7):
                    a_down[i, _rows(r, 16), pl.ds(col, n)] = ops[i]
                yield _tiles(*ops[:2], *ops[4:])

    def spread_keys(p, e, slot, release):
        for u in range(2):
            for d in range(DH):
                row = release(jnp.broadcast_to(kf[p, pl.ds(DH * e + d, 1), pl.ds(u * TH, TH)], (8, TH)))
                col = _cat([row[:, :VK]] * 16).T
                (kb0, kb1)[e][slot, d, pl.ds(u * VK, VK), :] = col
                yield [col[-8:]]

    def vector_scores(p, n, src, dst, track=None):
        e, t = divmod(n, NT)
        q = [_cat((jnp.broadcast_to(qf[p, t, pl.ds(DH * e + d, 1), pl.ds(col, TH)], (VB, TH))
                   for col in (0, TH)), 1) for d in range(DH)]
        for r in range(0, 2 * VK, VB):
            k = (kb0, kb1)[e][src, :, pl.ds(r, VB), :].reshape(DH * VB, 128)
            k = _cat([k, k], 1)
            for d in range(DH):
                term = k[VB * d:VB * (d + 1)] * q[d]
                s = s + term if d else term
                if d == DH - 1:
                    (sv.at[dst, n] if n else sv0.at[dst])[pl.ds(r, VB), :] = s
                    if track:
                        track(n, s)
                yield s

    def project(pace, t, j, m):
        def rhs(u, *pieces):
            where = ((1, 8), (7, 4))[u]
            return _unpack(_cat(
                xB[t, where[k // 3], _rows(64 * (k % 3), 64), :] if k < 6 else xB[t, 9, _rows(64 * u, 64), :]
                for k in pieces))

        out = []
        for u in range(2):
            r = [pace.dot(a_qkv[j, 7 * m + n], rhs(u, *pieces)) for n, pieces in enumerate(
                ((3, 4), (5, 6), (0, 1), (0, 2), (3, 4), (5, 6), (2, 1)))]
            out += [r[3] + (r[2] + (r[1] + r[0])), r[6] + (r[2] + (r[5] + r[4]))]
        out = _cat([_cat(out[0::2], 1), _cat(out[1::2], 1)])
        for x in range(NP // 2):
            p, blk = NP // 2 * m + x, out[2 * DH * x:2 * DH * (x + 1)]
            if j == 0:
                qf[p, t, pl.ds(0, 2 * DH), :] = blk * QSCALE
            elif j == 1:
                if t == 0:
                    kf[p, pl.ds(0, 2 * DH), :] = blk
                gap = jnp.zeros((8, TH), f32)
                kk[p, _rows(t * TH, TH), :] = _pack(_cat([blk[:, :TH], gap, blk[:, TH:], gap]).astype(bf16).T)
            else:
                for e in range(2):
                    ones = jnp.where(row32 == (0 if e else DH), 1.0, 0.0)
                    lo, inside = window(e)
                    vT[2 * p + e, :, pl.ds(t * TQ, TQ)] = _pack(jnp.where(inside, blk[lo:lo + HP], ones))

    def prologue():
        x = [(xT_hbm.at[:, pl.ds(t * TQ, TQ)], xT.at[t]) for t in range(NT)]
        wq, wkv = ((wqkv_hbm.at[:, cols], wqkv.at[:, cols]) for cols in (pl.ds(0, 512), pl.ds(512, 3 * D - 512)))
        groups = [x[:1], [wq, x[1]], [wkv], x[2:], [(wo_hbm, wo), (w2T_hbm, w2T), (w1_hbm, w1)], [(w3_hbm, w3)]]
        groups = [[pltpu.make_async_copy(src, dst, sems.at[i]) for src, dst in group]
                  for i, group in enumerate(groups)]
        starts, waits = {1: 3, 4: 4, 12: 5}, {1.5: 2, 5: 3, 14: 4, 19: 5}
        for cp in groups[0] + groups[1]:
            cp.start()
        groups[0][0].wait()
        for _ in normalize(0):
            pass
        groups[2][0].start()
        for cp in groups[1]:
            cp.wait()
        for _ in prepare_qkv(0):
            pass

        corner = xT[0, pl.ds(0, 16), pl.ds(0, 128)].astype(f32)[:8]
        pace = _Pacer(corner * corner < -1.0)
        order = [(0, 0), (1, 0), (0, 1), (1, 1), (0, 2), (1, 2)] + [(t, 1) for t in range(2, NT)]
        order += [(t, j) for t in range(2, NT) for j in (2, 0)]
        each = 49
        _, first, third, fourth = (each * n + 4 for n in waits)
        pace.add(normalize(1), 50, 0, each - 6)
        pace.add(prepare_qkv(2, pace.release), 18, 2 * each + 9, 4 * each - 8)
        for t in range(2, NT):
            last = each * order.index((t, 1)) - 6
            pace.add(normalize(t), 50, first, last)
            first = last
        down = prepare_down()
        pace.add(down, OUT_SPLIT, third, fourth - 14)
        pace.add(down, 56 - OUT_SPLIT, fourth, 24 * each - 8)
        out = prepare_o(pace.release)
        turns = _delayed([_first(out, 7), prepare_up(0, w1, pace.release), out, prepare_up(1, w3, pace.release)],
                         TURN_LAG)
        assert TURN_SPLIT <= 35 + 14 * NG
        pace.add(turns, TURN_SPLIT, third, fourth - TURN_END)
        pace.add(turns, 35 + 28 * NG + TURN_LAG - TURN_SPLIT, fourth, 24 * each - 2)
        pace.add(_delayed([spread_keys(0, 0, 0, pace.release)], 6), 2 * DH + 6, *(each * n for n in FIRST_KEYS))
        pace.add(([_tiles(s)[n % (VB // 4)]] for n, s in enumerate(vector_scores(0, 0, 0, 0))),
                 2 * VK // VB * DH, *(each * n for n in FIRST_SCORES))
        for n, (t, j) in enumerate(order):
            for m in range(2):
                project(pace, t, j, m)
                now = n + (m + 1) / 2
                if now in starts:
                    for cp in groups[starts[now]]:
                        cp.start()
                if now in waits:
                    for cp in groups[waits[now]]:
                        cp.wait()
                if waits.get(now) == 2:
                    for _ in prepare_qkv(1):
                        pass
        assert all(job[4] == job[1] for job in pace.jobs)

    program, score_plan, key_plan, activate = _plan()

    def pair(p, carry):
        put, get = p % 2, 1 - (p + 1) % 2
        never = [lax.broadcasted_iota(jnp.int32, (8, 128), 0) < -p - k for k in range(TIES + 2)]
        following = jnp.minimum(p + 1, NP - 1)
        peak = {}
        state = dict(slot=0, scores=0, keys=0, turn=0)

        def track(n, s):
            s = jnp.max(s.reshape(-1, 8, TQ), axis=0)
            peak[n] = jnp.maximum(peak[n], s) if n in peak else s

        def all_vector_scores():
            for n in range(1, 2 * NT):
                yield from vector_scores(p, n, get, put, track)
            yield from vector_scores(following, 0, 1 - get, 1 - put)

        def release(k):
            return lax.select(never[0], state["recent"], k) if "recent" in state else k

        def next_keys():
            yield from _delayed([spread_keys(p, 1, put, release)], KEY_LAG)
            yield from _delayed([spread_keys(following, 0, 1 - put, release)], KEY_LAG)

        def activation():
            for g in range(NG):
                for r in range(0, 128, 8):
                    gate, up = (_combine(mB[put, g, j, :, pl.ds(r, 8), :]) for j in range(2))
                    ops = _rhs_operands(*((a * b) * jnp.tanh(0.5 * a) + a * b for a, b in zip(gate, up)))
                    hB[put, g, :, pl.ds(r, 8), :] = jnp.stack(ops)
                    yield ops[6]

        side_scores, side_keys, side_hidden = all_vector_scores(), next_keys(), activation()

        def deadline():
            slot = state["slot"]
            state["slot"] += 1
            deps = [next(side_hidden)] if slot in activate else []
            while state["keys"] < key_plan[slot]:
                deps += next(side_keys)
                state["keys"] += 1
            if state["scores"] < score_plan[slot]:
                while state["scores"] < score_plan[slot]:
                    last = next(side_scores)
                    state["scores"] += 1
                for _ in range(TIES):
                    r, col = divmod(state["turn"] % (VB // 4), 2)
                    deps.append(last[8 * r:8 * r + 8, TH * col:TH * (col + 1)])
                    state["turn"] += 1
            return deps

        def lhs(x, paced):
            return _after(x, deadline, never, f32) if paced else _unpack(x)

        def queries(n):
            e, t = divmod(n, NT)
            lo, inside = window(e)
            win = jnp.where(inside, qf[p, t, pl.ds(lo, HP), :], 0.0)
            after = [jnp.zeros((8, TQ), f32)] * e
            return [_cat([jnp.zeros((64 * u + lo, TQ), f32)] * (u + e > 0) + [win] + after).astype(bf16)
                    for u in range(2)]

        def scores(n, t, q):
            lo, hi = _cut(t), _cut(t + 1)
            k = kk[p, _rows(lo, hi - lo), :]
            for u in range(2):
                s = _cat((_dot(lhs(k, u and x)[:, :q[u].shape[0]], q[u][:, x * TH:(x + 1) * TH])
                          for x in range(2)), 1)
                (s0, s1)[n % 2][put, u, pl.ds(lo, hi - lo), :] = s
                track(n, s)
            state["recent"] = s[:8, :128]

        def values(n, t, m):
            lo, hi = max(t * TH, VK), (t + 1) * TH
            parts = []
            for u in range(2):
                if t == 0:
                    parts.append((sv.at[put, n] if n else sv0.at[get])[pl.ds(u * VK, VK), :])
                parts.append((s0, s1)[n % 2][get, u, pl.ds(lo, hi - lo), :])
            weights = jnp.exp2(_cat(parts) - m).astype(bf16)
            return _dot(lhs(vT[2 * p + n // NT, :, pl.ds(t * TQ, TQ)], True), weights)

        track(0, sv0[put])
        results = []
        for ops in program:
            for unit, op in enumerate(ops):
                if op[0] == "scores":
                    _, n, t = op
                    if t == 0:
                        q = queries(n)
                    scores(n, t, q)
                elif op[0] == "values":
                    _, n, t = op
                    if t == 0:
                        assert state["scores"] >= n * 2 * VK // VB * DH
                        m = jnp.max(peak.pop(n), axis=0, keepdims=True)
                    acc = values(n, t, m) + acc if t else values(n, t, m)
                    if t == NT - 1:
                        total = 0 if n >= NT else DH
                        oF[p, n % NT, n // NT] = acc * (1.0 / acc[total:total + 1])
                elif op[0] == "up":
                    _, g, j, n = op
                    i, pieces = PASSES[n]
                    b = _cat(xB[p, i, _rows(64 * k, 64), :] if k < 3 else xB[p, 9, _rows(64 * REMAINDER[i], 64), :]
                             for k in pieces)
                    results.append(_dot(lhs(a_up[g, j, n], unit == 0), _unpack(b)))
                    state["recent"] = results[-1][:8]
                    for block, i, value in _finished(n, results):
                        mB[put, g, j, i, pl.ds(64 * block, 64), :] = value
                else:
                    _, i, r, k = op
                    part = _dot(lhs(a_down[i, _rows(r, D4), pl.ds(128 * k, 128)], unit == 0),
                                hB[put, k, i].astype(bf16))
                    state["recent"] = part[:8]
                    down = part + down if k else part
                    if k == NG - 1:
                        y[p, i, pl.ds(r, D4), :] = down
        assert not peak and all(next(side, None) is None for side in (side_scores, side_keys, side_hidden))
        return carry

    def epilogue():
        copies = []
        for t in range(NT):
            rows = []
            for p in range(NP):
                a, b = oF[p, t, 0], oF[p, t, 1]
                rows += [a[:HP - 8], jnp.where(row32[:8] < HP - DH, a[HP - 8:], b[:8]), b[8:]]
            o = _cat(rows)
            ops = _rhs_operands(*(o[r:r + KH, col:col + TH] for r in (0, KH) for col in (0, TH)))
            rhs = [_cat(ops[i][64 * k:64 * k + 64] if k < 3 else o[2 * KH:, TH * REMAINDER[i]:TH * (REMAINDER[i] + 1)]
                        for k in pieces).astype(bf16) for i, pieces in PASSES]
            for a_o, first, size in ((a_o0, 0, 64), (a_o1, 128, 48)):
                results, products = [], [{}, {}]
                for n in (*range(8), *range(16, NU), *range(8, 16)):
                    results.append(_dot(_unpack(a_o[n]), rhs[n]))
                    for block, i, value in _finished(n, results):
                        products[block][i] = value + 0.5 * y[t, i, pl.ds(first + block * size, size), :]
                out = [_combine(x) for x in products]
                out = _cat(_cat(out[block][2 * m:2 * m + 2], 1) for m in range(2) for block in range(2))
                span = pl.ds(2 * first, 4 * size)
                outb[t, span, :] = (xT[t, span, :].astype(f32) + out).astype(bf16)
                copies.append(pltpu.make_async_copy(
                    outb.at[t, span], outT_hbm.at[span, pl.ds(t * TQ, TQ)], sems.at[6]))
                copies[-1].start()
        for cp in copies:
            cp.wait()

    prologue()
    lax.fori_loop(0, NP, pair, 0)
    epilogue()


@jax.jit
def pallas_parallel_sum__softmax_full_mha__glu_gated_swiglu__prompt_kernel(
    A_x: jax.Array,
    A_wqkv: jax.Array,
    A_wo: jax.Array,
    B_x: jax.Array,
    B_w1: jax.Array,
    B_w3: jax.Array,
    B_w2: jax.Array,
):
    del B_x
    hbm = pl.BlockSpec(memory_space=pltpu.HBM)
    vm = pltpu.VMEM

    def packed(*shape):
        return vm(shape[:-2] + (shape[-2] // 2, shape[-1]), u32)

    scratch = [
        vm((NT, D, TQ), bf16), vm((D, 3 * D), bf16), vm((D, D), bf16),
        vm((D, F), bf16), vm((D, F), bf16), vm((D, F), bf16),
        packed(3, 16, D4, 128), packed(NG, 2, NU, 64, 128), packed(8, D2, F2),
        packed(NU, 64, 128), packed(NU + 3, 48, 128),
        packed(NT, 10, KH, TH), vm((NP, NT, 64, TQ), f32), vm((NP, 64, TQ), f32),
        packed(NP, S // 2, 128), vm((2, DH, 2 * VK, 128), f32),
        vm((2, DH, 2 * VK, 128), f32), packed(H, HP, S),
        vm((2, 2, S // 2, TQ), f32), vm((2, 2, S // 2, TQ), f32),
        vm((2, 2 * NT, 2 * VK, TQ), f32), vm((2, 2 * VK, TQ), f32),
        vm((2, NG, 2, 7, 128, TH), f32), vm((2, NG, 7, 128, TH), f32),
        vm((NP, NT, 2, HP, TQ), f32), vm((NT, 7, D2, TH), f32), vm((NT, D, TQ), bf16),
        pltpu.SemaphoreType.DMA((7,)),
    ]
    outT = pl.pallas_call(
        _kernel,
        out_shape=jax.ShapeDtypeStruct((D, S), bf16),
        in_specs=[hbm] * 6,
        out_specs=hbm,
        scratch_shapes=scratch,
        compiler_params=pltpu.CompilerParams(vmem_limit_bytes=100 * 2**20),
    )(A_x[0].T, A_wqkv, A_wo, B_w1, B_w3, B_w2.T)
    return outT.T[None]
```
